```python
import os as _os
_os.environ.setdefault("JAX_PLATFORMS", "cpu")
import jax
import jax.numpy as jnp

def _softmax(x, axis=-1):
    return jax.nn.softmax(x, axis=axis)
def _gelu(x):
    return jax.nn.gelu(x, approximate=True)
def _silu(x):
    return jax.nn.silu(x)
def _sigmoid(x):
    return jax.nn.sigmoid(x)
def _layernorm(x, axis=-1, eps=1e-5):
    m = jnp.mean(x, axis=axis, keepdims=True)
    v = jnp.var(x, axis=axis, keepdims=True)
    return (x - m) / jnp.sqrt(v + eps)
def _scatter_add(tgt, idx, src, axis=0):
    return tgt.at[idx].add(src)
def _segment_sum(src, seg, n):
    return jax.ops.segment_sum(src, seg, n)
class _Rng:
    def __init__(self, key):
        self._k = key
    def _next(self):
        self._k, sub = jax.random.split(self._k)
        return sub
    def normal(self, shape):
        return jax.random.normal(self._next(), shape, dtype=jnp.bfloat16)
    def randint(self, lo, hi, shape):
        return jax.random.randint(self._next(), shape, lo, hi, dtype=jnp.int32)
    def uniform(self, shape, lo=0.0, hi=1.0):
        return jax.random.uniform(self._next(), shape, jnp.bfloat16, lo, hi)
    def permutation(self, n):
        return jax.random.permutation(self._next(), n)


kernel_name = 'sequential_preLN__spectral_gfnet__glu_gated_bilinear__prompt'

def setup_inputs():
    _rng = _Rng(jax.random.key(int.from_bytes(__import__("os").urandom(4), "little")))
    _w = (lambda a: (lambda t: t.astype(jnp.bfloat16) if jnp.issubdtype(t.dtype, jnp.floating) else t)(jnp.asarray(a)))
    def _A_setup():
        B, S, D = 1, 2048, 448
        Df = D // 2 + 1
        return {
            "x": _w((lambda *s: _rng.normal(s) * 0.05)(B, S, D)),
            "w_r": _w((lambda *s: _rng.normal(s) * 0.2)(S, Df) * 0.02),
            "w_i": _w((lambda *s: _rng.normal(s) * 0.2)(S, Df) * 0.02),
        }
    _A_in = _A_setup()

    def _B_setup():
        B, S, D, F = 1, 2048, 448, 1792
        return {
            "x": _w((lambda *s: _rng.normal(s) * 0.05)(B, S, D)),
            "w_gate": _w((lambda *s: _rng.normal(s) * 0.05)(D, F) * (D ** -0.5)),
            "w_up": _w((lambda *s: _rng.normal(s) * 0.05)(D, F) * (D ** -0.5)),
            "w_down": _w((lambda *s: _rng.normal(s) * 0.05)(F, D) * (F ** -0.5)),
        }
    _B_in = _B_setup()

    return {
        "A_x": _A_in["x"],
        "A_w_r": _A_in["w_r"],
        "A_w_i": _A_in["w_i"],
        "B_x": _B_in["x"],
        "B_w_gate": _B_in["w_gate"],
        "B_w_up": _B_in["w_up"],
        "B_w_down": _B_in["w_down"],
    }

def reference(A_x, A_w_r, A_w_i, B_x, B_w_gate, B_w_up, B_w_down):
    def _A_ref(x, w_r, w_i):
        B, S, D = x.shape
        X = (lambda x, axes=(-2,-1): jnp.fft.rfft2(x.astype(jnp.float32), axes=axes))(x, axes=(-2, -1))
        W = w_r + 1j * w_i
        X = X * W
        y = (lambda x, s, axes=(-2,-1): jnp.fft.irfft2(x, s=s, axes=axes).astype(jnp.bfloat16))(X, (S, D), axes=(-2, -1))
        return y

    def _B_ref(x, w_gate, w_up, w_down):
        g = jnp.einsum("bsd,df->bsf", x, w_gate)
        u = jnp.einsum("bsd,df->bsf", x, w_up)
        h = g * u
        return jnp.einsum("bsf,fd->bsd", h, w_down)

    x = A_x
    h = x + _A_ref(_layernorm(x, axis=-1), A_w_r, A_w_i)
    h2 = h + _B_ref(_layernorm(h, axis=-1), B_w_gate, B_w_up, B_w_down)
    return h2
```

```python
import contextlib
import math

import jax
import jax.numpy as jnp
import ml_dtypes
import numpy as np
from jax import lax
import jax.experimental.pallas as pl
import jax.experimental.pallas.tpu as pltpu

BF = ml_dtypes.bfloat16
S, D, F = 2048, 448, 1792
H = 224

def kd_order():
    r=np.arange(112); v=r//16; i=(r%16)//2; half=r%2
    base=2*(16*v+8*half+i)
    kE=base.copy(); kE[kE==0]=224
    kO=base+1
    return kE,kO

def _cs(num,den):
    num=np.mod(num,den)
    a=2*np.pi*num/den
    c=np.cos(a); s=np.sin(a)
    c=np.where(np.abs(c)<1e-12,0,c); s=np.where(np.abs(s)<1e-12,0,s)
    return c,s

def d_fwd():
    out=np.zeros((2,224,256))
    d2=np.arange(H)
    for t,k in enumerate(kd_order()):
        c,s=_cs(k[:,None]*d2[None,:],D)
        out[t,:112,:H]=c; out[t,112:,:H]=-s
    return out

def d_inv():
    out=np.zeros((2,H,256))
    d2=np.arange(H)
    for t,k in enumerate(kd_order()):
        ck=np.where(k==224,1.0,2.0)/D
        c,s=_cs(d2[:,None]*k[None,:],D)
        out[t,:,:112]=c*ck; out[t,:,128:240]=-s*ck
    return out

def w_perm():
    L=np.zeros((128,128));
    for k1 in range(16):
        for l in range(8): L[8*k1+l,k1+16*l]=1
    return L


def d_inv_scaled():
    return d_inv()/S

def add(a,b): return (a[0]+b[0],a[1]+b[1])
def sub(a,b): return (a[0]-b[0],a[1]-b[1])
def fft4(x,inv):
    t0=add(x[0],x[2]); t1=sub(x[0],x[2]); t2=add(x[1],x[3]); t3=sub(x[1],x[3])
    mi=(t1[0]+t3[1],t1[1]-t3[0]); pi=(t1[0]-t3[1],t1[1]+t3[0])
    return [add(t0,t2), pi if inv else mi, sub(t0,t2), mi if inv else pi]
def tw16(x,e,inv):
    e%=16
    if e==0: return x
    if e==4:
        return (-x[1],x[0]) if inv else (x[1],-x[0])
    c=math.cos(2*math.pi*e/16); s=math.sin(2*math.pi*e/16)*(1 if inv else -1)
    if e in (2,6):
        r=abs(c)
        sc=1 if c>0 else -1; ss=1 if s>0 else -1
        a,b=x
        re=(a if sc>0 else -a); re2=(-b if ss>0 else b)
        if sc>0 and ss>0: return ((a-b)*r,(a+b)*r)
        if sc>0 and ss<0: return ((a+b)*r,(b-a)*r)
        if sc<0 and ss>0: return ((a+b)*(-r),(a-b)*r)
        return ((b-a)*r,(a+b)*(-r))
    a,b=x
    return (a*c-b*s,b*c+a*s)
def fft16(x,inv):
    t=[None]*16
    for a0 in range(4):
        y=fft4([x[4*a1+a0] for a1 in range(4)],inv)
        for k0 in range(4): t[4*a0+k0]=tw16(y[k0],a0*k0,inv)
    out=[None]*16
    for k0 in range(4):
        y=fft4([t[4*a0+k0] for a0 in range(4)],inv)
        for k in range(4): out[k0+4*k]=y[k]
    return out


bf=jnp.bfloat16; f32=jnp.float32; u32=jnp.uint32
NT=(((1,),(1,)),((),())); TN=(((0,),(0,)),((),()))
def dNT(a,b): return lax.dot_general(a,b,NT,preferred_element_type=f32)
def dTN(a,b): return lax.dot_general(a,b,TN,preferred_element_type=f32)
def dNN(a,b): return jnp.dot(a,b,preferred_element_type=f32)
T=512
XCH=[(0,128),(128,512),(512,1024),(1024,1536),(1536,1792),(1792,1920),(1920,2048)]
SCOPES=False
def scope(n): return jax.named_scope(n) if SCOPES else contextlib.nullcontext()

def kernel(x_h,wr_h,wi_h,wg_h,wu_h,wd_h,ld_h,li_h,pm_h,o_h,
           xs,wraw,nyq,wg,wu,wd,ld,li,mf,pm,Z,Wp,U,lnb,hb,ob,sem):
    cp=pltpu.make_async_copy
    si=iter(range(40))
    def mk(s,d): return cp(s,d,sem.at[next(si)])
    d_ld=mk(ld_h,ld)
    d_x=[mk(x_h.at[:,a:b],xs.at[:,a:b]) for a,b in XCH]
    d_pm=mk(pm_h,pm)
    d_nq=[mk(wr_h.at[224:225,:],nyq.at[0]),mk(wi_h.at[224:225,:],nyq.at[1])]
    d_w=[[mk(w.at[0:224,512*c:512*c+512],wraw.at[i,:,512*c:512*c+512]) for i,w in enumerate((wr_h,wi_h))] for c in range(4)]
    d_li=mk(li_h,li); d_wg=mk(wg_h,wg); d_wu=mk(wu_h,wu); d_wd=mk(wd_h,wd)
    d_ld.start()
    for d in d_x: d.start()
    d_pm.start()
    for d in d_nq: d.start()
    for c in range(4):
        for d in d_w[c]: d.start()
    d_li.start(); d_wg.start(); d_wu.start(); d_wd.start()
    with scope("mbuild"):
        r=lax.broadcasted_iota(jnp.int32,(128,128),0); c_=lax.broadcasted_iota(jnp.int32,(128,128),1)
        ang=((r*c_)&127).astype(f32)*(2*math.pi/128)
        c0=jnp.cos(ang); s0=-jnp.sin(ang)
        r2=lax.broadcasted_iota(jnp.int32,(16,128),0); c2=lax.broadcasted_iota(jnp.int32,(16,128),1)
        a2=(r2*c2).astype(f32)*(2*math.pi/2048)
        tc=jnp.cos(a2); ts=-jnp.sin(a2)
        for k1 in range(16):
            if k1==0: C,Sn=c0,s0
            else:
                a=tc[k1:k1+1,:]; b=ts[k1:k1+1,:]
                C=c0*a-s0*b; Sn=c0*b+s0*a
            for j,m in enumerate((C,Sn,C+Sn)): mf[k1,128*j:128*j+128,:]=m.astype(bf)
    def f2_tile(ai):
        cs=slice(128*ai,128*ai+128)
        lo=xs[0:H,cs].astype(f32); hi=xs[H:D,cs].astype(f32)
        o=lo-hi; obf=o.astype(bf); so=jnp.sum(o*o,axis=0,keepdims=True)
        e=lo+hi; me=jnp.sum(e,axis=0,keepdims=True)*(1.0/H); ec=e-me; ebf=ec.astype(bf)
        ss=so+jnp.sum(ec*ec,axis=0,keepdims=True)
        rr=lax.rsqrt(ss*(0.5/D)+1e-5)
        for t,a in enumerate((ebf,obf)):
            z=dNN(ld[t],a)*rr
            Z[t,0,ai]=z[:112]; Z[t,1,ai]=z[112:]
    for i,(a,b) in enumerate(XCH):
        with scope(f"waitx{i}"):
            if i==0: d_ld.wait()
            d_x[i].wait()
        with scope(f"F2_{i}"):
            for ai in range(a//128,b//128): f2_tile(ai)
    def f3(t):
        for g in range(14):
            xin=[(Z[t,0,a,8*g:8*g+8,:],Z[t,1,a,8*g:8*g+8,:]) for a in range(16)]
            y=fft16(xin,False)
            for k in range(16):
                Z[t,0,k,8*g:8*g+8,:]=y[k][0]; Z[t,1,k,8*g:8*g+8,:]=y[k][1]
    ww=wraw.bitcast(u32)
    sub0=lax.broadcasted_iota(jnp.int32,(8,512),0)==0
    def wprep(c):
        cs=slice(512*c,512*c+512)
        for ri in range(2):
            nq=lax.shift_right_logical(pltpu.bitcast(nyq[ri,:,cs].astype(f32),u32),jnp.uint32(16))
            e=[];o=[]
            for v in range(7):
                A=ww[ri,16*v:16*v+8,cs]; B=ww[ri,16*v+8:16*v+16,cs]
                lo=A&jnp.uint32(0xffff)
                if v==0: lo=jnp.where(sub0,nq,lo)
                e.append(lo|(B<<jnp.uint32(16)))
                o.append((A>>jnp.uint32(16))|(B&jnp.uint32(0xffff0000)))
            zpad=jnp.zeros((8,512),u32)
            tiles=[]
            for t,l in enumerate((e,o)):
                big=pltpu.bitcast(jnp.concatenate(l+[zpad],axis=0),bf)
                for p in range(4): tiles.append(big[:,128*p:128*p+128])
            r=dNT(pm[...],jnp.concatenate(tiles,axis=0))
            for t in range(2):
                for p in range(4):
                    j=4*t+p; pp=4*c+p
                    for k1 in range(16):
                        Wp[ri,t,k1,8*pp:8*pp+8,:]=r[8*k1:8*k1+8,128*j:128*j+128]
    zf=jnp.zeros((16,128),f32)
    def pad2(x0,x1): return jnp.concatenate([x0,zf,x1,zf],axis=0).astype(bf)
    def stA(k1):
        a0,a1=Z[0,0,k1],Z[1,0,k1]; b0,b1=Z[0,1,k1],Z[1,1,k1]
        m1=dNT(mf[k1,0:128,:],pad2(a0,a1)); m2=dNT(mf[k1,128:256,:],pad2(b0,b1)); m3=dNT(mf[k1,256:384,:],pad2(a0+b0,a1+b1))
        return m1-m2, m3-m1-m2
    def stB(k1,Y):
        Yr,Yi=Y
        Wr=jnp.concatenate([Wp[0,0,k1],Wp[0,1,k1]],axis=1); Wi=jnp.concatenate([Wp[1,0,k1],Wp[1,1,k1]],axis=1)
        yr=Yr*Wr-Yi*Wi; yi=Yr*Wi+Yi*Wr
        m1=dTN(mf[k1,0:128,:],yr.astype(bf)); m2=dTN(mf[k1,128:256,:],yi.astype(bf)); m3=dTN(mf[k1,256:384,:],(yr-yi).astype(bf))
        ur=m1+m2; ui=m1-m2-m3
        for t in range(2):
            U[0,t,128*k1:128*k1+128,:]=ur[:,128*t:128*t+128]
            U[1,t,128*k1:128*k1+128,:]=ui[:,128*t:128*t+128]
    with scope("F3E"): f3(0)
    Y=[]
    for c in range(4):
        with scope(f"waitw{c}"):
            if c==0: d_pm.wait(); d_nq[0].wait(); d_nq[1].wait()
            d_w[c][0].wait(); d_w[c][1].wait()
        with scope(f"wprep{c}"):
            wprep(c)
            if c==0: f3(1)
            else: Y.append(stA(c-1))
    with scope("F46"):
        for i in range(16):
            while len(Y)<min(16,i+3): Y.append(stA(len(Y)))
            stB(i,Y[i])
    with scope("F7"):
        for t in range(2):
            for g in range(16):
                xin=[(U[0,t,128*k+8*g:128*k+8*g+8,:],U[1,t,128*k+8*g:128*k+8*g+8,:]) for k in range(16)]
                y=fft16(xin,True)
                for a in range(16):
                    U[0,t,128*a+8*g:128*a+8*g+8,:]=y[a][0]; U[1,t,128*a+8*g:128*a+8*g+8,:]=y[a][1]
    with scope("waitwt"):
        d_li.wait(); d_wg.wait(); d_wu.wait(); d_wd.wait()
    outs=[]
    def prep(c):
        rs=slice(c*T,(c+1)*T)
        Vs=[]
        for t in range(2):
            V=jnp.concatenate([U[0,t,rs,:],U[1,t,rs,:]],axis=1).astype(bf)
            Vs.append(dNT(li[t],V))
        x=xs[:,rs].astype(f32)
        h=jnp.concatenate([x[:H]+(Vs[0]+Vs[1]),x[H:]+(Vs[0]-Vs[1])],axis=0).astype(bf)
        hb[c%3]=h
        hf=h.astype(f32)
        m=jnp.sum(hf,axis=0,keepdims=True)*(1.0/D)
        hc=hf-m
        v=jnp.sum(hc*hc,axis=0,keepdims=True)*(1.0/D)
        ln=hc*lax.rsqrt(v+1e-5)
        lnb[c%2]=ln.T.astype(bf)
    def ffn(c):
        rs=slice(c*T,(c+1)*T)
        xl=lnb[c%2]
        g=dNN(xl,wg[...]); u=dNN(xl,wu[...])
        hh=(g*u).astype(bf)
        o=dNT(wd[...],hh)
        if c>=2: outs[c-2].wait()
        ob[c%2]=(hb[c%3].astype(f32)+o).astype(bf)
        d=mk(ob.at[c%2],o_h.at[:,rs]); d.start(); outs.append(d)
    with scope("prep0"): prep(0)
    for c in range(4):
        with scope(f"back{c}"):
            if c<3: prep(c+1)
            ffn(c)
    with scope("waitout"):
        outs[2].wait(); outs[3].wait()

@jax.jit
def pallas_sequential_preLN__spectral_gfnet__glu_gated_bilinear__prompt_kernel(A_x,A_w_r,A_w_i,B_x,B_w_gate,B_w_up,B_w_down):
    xT=A_x.reshape(S,D).T; wrT=A_w_r.T; wiT=A_w_i.T; wdT=B_w_down.T
    Ld=jnp.asarray(d_fwd()[:,:,:H].astype(BF)); Li=jnp.asarray(d_inv_scaled().astype(BF))
    Pm=jnp.asarray(w_perm().astype(BF))
    anyspec=pl.BlockSpec(memory_space=pltpu.HBM)
    out=pl.pallas_call(kernel,
        out_shape=jax.ShapeDtypeStruct((D,S),bf),
        in_specs=[anyspec]*9,out_specs=anyspec,
        scratch_shapes=[pltpu.VMEM((D,S),bf),pltpu.VMEM((2,224,S),bf),pltpu.VMEM((2,1,S),bf),
            pltpu.VMEM((D,F),bf),pltpu.VMEM((D,F),bf),pltpu.VMEM((D,F),bf),
            pltpu.VMEM((2,224,H),bf),pltpu.VMEM((2,H,256),bf),
            pltpu.VMEM((16,384,128),bf),pltpu.VMEM((128,128),bf),
            pltpu.VMEM((2,2,16,112,128),f32),pltpu.VMEM((2,2,16,128,128),f32),pltpu.VMEM((2,2,S,128),f32),
            pltpu.VMEM((2,T,D),bf),pltpu.VMEM((3,D,T),bf),pltpu.VMEM((2,D,T),bf),
            pltpu.SemaphoreType.DMA((40,))],
        compiler_params=pltpu.CompilerParams(vmem_limit_bytes=100*1024*1024),
    )(xT,wrT,wiT,B_w_gate,B_w_up,wdT,Ld,Li,Pm)
    return out.T.reshape(1,S,D)
```

```python
import contextlib
import functools
import math

import jax
import jax.numpy as jnp
import ml_dtypes
import numpy as np
from jax import lax
import jax.experimental.pallas as pl
import jax.experimental.pallas.tpu as pltpu

BF = ml_dtypes.bfloat16
S, D, F = 2048, 448, 1792
H = 224

def kd_order():
    r=np.arange(112); v=r//16; i=(r%16)//2; half=r%2
    base=2*(16*v+8*half+i)
    kE=base.copy(); kE[kE==0]=224
    kO=base+1
    return kE,kO

def _cs(num,den):
    num=np.mod(num,den)
    a=2*np.pi*num/den
    c=np.cos(a); s=np.sin(a)
    c=np.where(np.abs(c)<1e-12,0,c); s=np.where(np.abs(s)<1e-12,0,s)
    return c,s

def d_inv():
    out=np.zeros((2,H,256))
    d2=np.arange(H)
    for t,k in enumerate(kd_order()):
        ck=np.where(k==224,1.0,2.0)/D
        c,s=_cs(d2[:,None]*k[None,:],D)
        out[t,:,:112]=c*ck; out[t,:,128:240]=-s*ck
    return out

def kd_order2():
    kE=2*np.arange(112); kE[0]=224
    kO=2*np.arange(112)+1
    return kE,kO

def d_fwd2():
    out=np.zeros((2,224,H)); d2=np.arange(H)
    for t,k in enumerate(kd_order2()):
        c,s=_cs(k[:,None]*d2[None,:],D)
        out[t,:112]=c; out[t,112:]=-s
    return out

def d_inv2():
    out=np.zeros((2,H,256)); d2=np.arange(H)
    for t,k in enumerate(kd_order2()):
        ck=np.where(k==224,1.0,2.0)/(D*S)
        c,s=_cs(d2[:,None]*k[None,:],D)
        out[t,:,:112]=c*ck; out[t,:,128:240]=-s*ck
    return out


def d_fwd3():
    kE,kO=kd_order2()
    d3=np.arange(112)
    lE=np.zeros((2,112,112))
    for j,k in enumerate((kE[0::2],kE[1::2])):
        c,s=_cs(k[:,None]*d3[None,:],D)
        lE[j,:56]=c; lE[j,56:]=-s
    d2=np.arange(H)
    c,s=_cs(kO[:,None]*d2[None,:],D)
    lO=np.concatenate([c,-s],0)
    return lE,lO

def d_inv3():
    kE,kO=kd_order2()
    sc=1.0/(D*S)
    out=np.zeros((4,112,128))
    d3=np.arange(112)[:,None]
    for j,k in enumerate((kE[0::2],kE[1::2])):
        ck=np.where(k==224,1.0,2.0)*sc
        c,s=_cs(d3*k[None,:],D)
        out[j,:,0:112:2]=c*ck; out[j,:,1:112:2]=-s*ck
    d2=np.arange(56)
    for which in (0,1):
        for l in range(112):
            m=l%4
            if which==0: i,part=[(l,0),(l-1,1),(l+1,1),(l,0)][m]
            else:        i,part=[(l+1,1),(l,0),(l,0),(l-1,1)][m]
            k=kO[i]; c,s=_cs(d2*k,D)
            sg=1.0 if k%8 in (1,3) else -1.0
            if part==0: re,im=c,s*sg
            else:       re,im=-s,c*sg
            out[2+which,:56,l]=2*sc*re; out[2+which,56:,l]=2*sc*im
    return out


def add(a,b): return (a[0]+b[0],a[1]+b[1])
def sub(a,b): return (a[0]-b[0],a[1]-b[1])
def fft4(x,inv):
    t0=add(x[0],x[2]); t1=sub(x[0],x[2]); t2=add(x[1],x[3]); t3=sub(x[1],x[3])
    mi=(t1[0]+t3[1],t1[1]-t3[0]); pi=(t1[0]-t3[1],t1[1]+t3[0])
    return [add(t0,t2), pi if inv else mi, sub(t0,t2), mi if inv else pi]
def tw16(x,e,inv):
    e%=16
    if e==0: return x
    if e==4:
        return (-x[1],x[0]) if inv else (x[1],-x[0])
    c=math.cos(2*math.pi*e/16); s=math.sin(2*math.pi*e/16)*(1 if inv else -1)
    if e in (2,6):
        r=abs(c)
        sc=1 if c>0 else -1; ss=1 if s>0 else -1
        a,b=x
        re=(a if sc>0 else -a); re2=(-b if ss>0 else b)
        if sc>0 and ss>0: return ((a-b)*r,(a+b)*r)
        if sc>0 and ss<0: return ((a+b)*r,(b-a)*r)
        if sc<0 and ss>0: return ((a+b)*(-r),(a-b)*r)
        return ((b-a)*r,(a+b)*(-r))
    a,b=x
    return (a*c-b*s,b*c+a*s)
def fft16(x,inv):
    t=[None]*16
    for a0 in range(4):
        y=fft4([x[4*a1+a0] for a1 in range(4)],inv)
        for k0 in range(4): t[4*a0+k0]=tw16(y[k0],a0*k0,inv)
    out=[None]*16
    for k0 in range(4):
        y=fft4([t[4*a0+k0] for a0 in range(4)],inv)
        for k in range(4): out[k0+4*k]=y[k]
    return out


bf=jnp.bfloat16; f32=jnp.float32; u32=jnp.uint32
NT=(((1,),(1,)),((),())); TN=(((0,),(0,)),((),()))
def dNT(a,b): return lax.dot_general(a,b,NT,preferred_element_type=f32)
def dTN(a,b): return lax.dot_general(a,b,TN,preferred_element_type=f32)
def dNN(a,b): return jnp.dot(a,b,preferred_element_type=f32)
T=512; TH=T//2; FH=F//2
XCH=[(0,4),(4,8),(8,12),(12,16)]
BM="1"
TP="000"
OPT="guI"
PREP="b32"
LN1="0"
TIE="0"
SCOPES=False
def scope(n): return jax.named_scope(n) if SCOPES else contextlib.nullcontext()

def kernel(x_h,wr_h,wi_h,wg_h,wu_h,wd_h,ld_h,li_h,le_h,l3_h,o_h,
           xs,wraw,nyq,wg,wu,wd,ld,li,mf,Z,Y,Wt,U,ve,lnf,al,hb,ob,bw,aw,bc,le,l3,sem):
    cp=pltpu.make_async_copy
    si=iter(range(80))
    def mk(s,d): return cp(s,d,sem.at[next(si)])
    d_ld=mk(ld_h,ld); d_le=mk(le_h,le); d_l3=mk(l3_h,l3)
    d_x=[mk(x_h.at[:,128*a:128*b],xs.at[:,128*a:128*b]) for a,b in XCH]
    d_nq=[mk(wr_h.at[224:225,:],nyq.at[0]),mk(wi_h.at[224:225,:],nyq.at[1])]
    d_w=[[mk(w.at[0:224,512*c:512*c+512],wraw.at[i,:,512*c:512*c+512]) for i,w in enumerate((wr_h,wi_h))] for c in range(4)]
    d_li=mk(li_h,li)
    GUC=[(0,7)]
    d_gu=[[mk(w.at[:,256*a:256*b],v.at[:,256*a:256*b]) for w,v in ((wg_h,wg),(wu_h,wu))] for a,b in GUC]
    d_wd=mk(wd_h,wd)
    d_ld.start()
    for d in d_x: d.start()
    for d in d_nq: d.start()
    for c in range(4):
        for d in d_w[c]: d.start()
    d_li.start(); d_l3.start()
    for ds in d_gu:
        for d in ds: d.start()
    d_wd.start()
    with scope("P0mbuild"):
        r=lax.broadcasted_iota(jnp.int32,(128,128),0); c_=lax.broadcasted_iota(jnp.int32,(128,128),1)
        ang=((r*c_)&127).astype(f32)*(2*math.pi/128)
        c0=jnp.cos(ang); s0=-jnp.sin(ang)
        r2=lax.broadcasted_iota(jnp.int32,(16,128),0); c2=lax.broadcasted_iota(jnp.int32,(16,128),1)
        a2=(r2*c2).astype(f32)*(2*math.pi/2048)
        tc=jnp.cos(a2); ts=-jnp.sin(a2)
        for k1 in range(16):
            if k1==0: C,Sn=c0,s0
            else:
                a=tc[k1:k1+1,:]; b=ts[k1:k1+1,:]
                C=c0*a-s0*b; Sn=c0*b+s0*a
            for j,m in enumerate((C,Sn-C,C+Sn) if 'g' in OPT else (C,Sn,C+Sn)):
                if 'u' in OPT: mf[k1,64*j:64*j+64,:]=pltpu.bitcast(m.astype(bf),u32)
                else: mf[k1,128*j:128*j+128,:]=m.astype(bf)
    def pre(ai):
        cs=slice(128*ai,128*ai+128)
        lo=xs[0:H,cs].astype(f32); hi=xs[H:D,cs].astype(f32)
        o=lo-hi; obf=o.astype(bf); e=lo+hi
        so=jnp.sum(o*o+e*e,axis=0,keepdims=True) if (LN1=='1' and 'R' not in OPT) else jnp.sum(o*o,axis=0,keepdims=True)
        if 'R' in OPT:
            eo=e[:112]-e[112:]; ee=e[:112]+e[112:]
            m2=jnp.sum(ee,axis=0,keepdims=True)*(1.0/112); ee=ee-m2
            ss=so+0.5*jnp.sum(ee*ee+eo*eo,axis=0,keepdims=True)
            return (ee.astype(bf),eo.astype(bf)),obf,lax.rsqrt(ss*(0.5/D)+1e-5)
        if LN1=='1':
            se=jnp.sum(e,axis=0,keepdims=True); me=se*(1.0/H); ebf=(e-me).astype(bf)
            ss=jnp.maximum(so-se*me,0.0)
            return ebf,obf,lax.rsqrt(ss*(0.5/D)+1e-5)
        me=jnp.sum(e,axis=0,keepdims=True)*(1.0/H); ec=e-me; ebf=ec.astype(bf)
        ss=so+jnp.sum(ec*ec,axis=0,keepdims=True)
        return ebf,obf,lax.rsqrt(ss*(0.5/D)+1e-5)
    def post(ai,ebf,obf,rr):
        if 'R' in OPT:
            for j in range(2):
                z=dNN(le[j],ebf[j])*rr
                Z[0,0,ai,pl.ds(j,56,stride=2),:]=z[:56]; Z[0,1,ai,pl.ds(j,56,stride=2),:]=z[56:]
        else:
            z=dNN(ld[0],ebf)*rr
            Z[0,0,ai]=z[:112]; Z[0,1,ai]=z[112:]
        z=dNN(ld[1],obf)*rr
        Z[1,0,ai]=z[:112]; Z[1,1,ai]=z[112:]
    with scope("P1F2"):
        for i,(a,b) in enumerate(XCH):
            if i==0: d_ld.wait()
            d_x[i].wait()
            for ai in range(a,b): post(ai,*pre(ai))
    def f3(t,gs=range(14)):
        for g in gs:
            xin=[(Z[t,0,a,8*g:8*g+8,:],Z[t,1,a,8*g:8*g+8,:]) for a in range(16)]
            y=fft16(xin,False)
            for k in range(16):
                Z[t,0,k,8*g:8*g+8,:]=y[k][0]; Z[t,1,k,8*g:8*g+8,:]=y[k][1]
    def loc(k): return 4*(k%4)+k//4
    def p1(ld_,st_,a0,inv):
        y=fft4([ld_(4*a1+a0) for a1 in range(4)],inv)
        for k0 in range(4): st_(4*k0+a0,tw16(y[k0],a0*k0,inv))
    def p2(ld_,st_,k0,inv):
        y=fft4([ld_(4*k0+a0) for a0 in range(4)],inv)
        for k in range(4): st_(4*k0+k,y[k])
    def zio(t,g):
        def l(a): return (Z[t,0,a,8*g:8*g+8,:],Z[t,1,a,8*g:8*g+8,:])
        def s_(a,v): Z[t,0,a,8*g:8*g+8,:]=v[0]; Z[t,1,a,8*g:8*g+8,:]=v[1]
        return l,s_
    def uio(t,g):
        def l(a): return (U[0,t,128*a+8*g:128*a+8*g+8,:],U[1,t,128*a+8*g:128*a+8*g+8,:])
        def s_(a,v): U[0,t,128*a+8*g:128*a+8*g+8,:]=v[0]; U[1,t,128*a+8*g:128*a+8*g+8,:]=v[1]
        return l,s_
    def tasks2(io,t,ng,inv):
        out=[]
        for g in range(ng):
            l,s_=io(t,g)
            out+=[functools.partial(p1,l,s_,a0,inv) for a0 in range(4)]
            out+=[functools.partial(p2,l,s_,k0,inv) for k0 in range(4)]
        return out
    def wt(c):
        for ri in range(2):
            for p in range(4*c,4*c+4):
                cs=slice(128*p,128*p+128)
                w=pltpu.bitcast(wraw[ri,:,cs],u32)
                nq=lax.shift_right_logical(pltpu.bitcast(nyq[ri,:,cs].astype(f32),u32),jnp.uint32(16))
                r0=lax.broadcasted_iota(jnp.int32,(8,128),0)==0
                first=jnp.where(r0,(w[0:8]&jnp.uint32(0xffff0000))|nq,w[0:8])
                tile=jnp.concatenate([first,w[8:112],jnp.zeros((16,128),u32)],axis=0)
                tt=tile.T
                for g in range(16):
                    r_=17*(8*p+g//2)+8*(g%2)
                    if 'w' in OPT:
                        v=tt[8*g:8*g+8]
                        Wt[ri,0,r_:r_+8,:]=pltpu.bitcast(v<<jnp.uint32(16),f32); Wt[ri,1,r_:r_+8,:]=pltpu.bitcast(v&jnp.uint32(0xffff0000),f32)
                    else: Wt[ri,r_:r_+8,:]=tt[8*g:8*g+8]
    zf=jnp.zeros((16,128),f32)
    def pad(x): return jnp.concatenate([x,zf],axis=0).astype(bf)
    def mfl(k1,j):
        return pltpu.bitcast(mf[k1,64*j:64*j+64,:],bf) if 'u' in OPT else mf[k1,128*j:128*j+128,:]
    def stA(t,k1):
        kk=loc(k1) if (t==1 and TP[0]=='1') else k1
        a=Z[t,0,kk]; b=Z[t,1,kk]
        if 'g' in OPT:
            m1=dNT(mfl(k1,0),pad(a+b)); m2=dNT(mfl(k1,1),pad(a)); m3=dNT(mfl(k1,2),pad(b))
            Y[0,t,k1]=m1-m3; Y[1,t,k1]=m1+m2
        else:
            m1=dNT(mfl(k1,0),pad(a)); m2=dNT(mfl(k1,1),pad(b)); m3=dNT(mfl(k1,2),pad(a+b))
            Y[0,t,k1]=m1-m2; Y[1,t,k1]=m3-m1-m2
    def stB(t,k1):
        if 'w' in OPT: w=[Wt[ri,t,pl.ds(k1,128,stride=17),:] for ri in range(2)]
        else: w=[Wt[ri,pl.ds(k1,128,stride=17),:] for ri in range(2)]
        def half(x): return pltpu.bitcast(x<<jnp.uint32(16),f32) if t==0 else pltpu.bitcast(x&jnp.uint32(0xffff0000),f32)
        Wr,Wi=(w[0],w[1]) if 'w' in OPT else (half(w[0]),half(w[1])); Yr=Y[0,t,k1]; Yi=Y[1,t,k1]
        yr=Yr*Wr-Yi*Wi; yi=Yr*Wi+Yi*Wr
        if 'g' in OPT:
            m1=dTN(mfl(k1,0),(yr+yi).astype(bf)); m2=dTN(mfl(k1,1),yi.astype(bf)); m3=dTN(mfl(k1,2),yr.astype(bf))
            U[0,t,128*k1:128*k1+128,:]=m1+m2; U[1,t,128*k1:128*k1+128,:]=m1-m3
        else:
            m1=dTN(mfl(k1,0),yr.astype(bf)); m2=dTN(mfl(k1,1),yi.astype(bf)); m3=dTN(mfl(k1,2),(yr-yi).astype(bf))
            U[0,t,128*k1:128*k1+128,:]=m1+m2; U[1,t,128*k1:128*k1+128,:]=m1-m2-m3
    def f7g(t,g):
        xin=[(U[0,t,128*k+8*g:128*k+8*g+8,:],U[1,t,128*k+8*g:128*k+8*g+8,:]) for k in range(16)]
        y=fft16(xin,True)
        for a in range(16):
            U[0,t,128*a+8*g:128*a+8*g+8,:]=y[a][0]; U[1,t,128*a+8*g:128*a+8*g+8,:]=y[a][1]
    lane=lax.broadcasted_iota(jnp.int32,(128,128),1)
    leven=(lane&1)==0; m03=((lane&3)==0)|((lane&3)==3)
    def dinv(t,ai):
        aj=loc(ai) if TP[1+t]=='1' else ai
        rs=slice(128*aj,128*aj+128)
        re=U[0,t,rs,:]; im=U[1,t,rs,:]
        if t==0 and 'I' in OPT:
            T0=jnp.where(leven,re,pltpu.roll(im,1,1)).astype(bf); T2=jnp.where(leven,pltpu.roll(re,127,1),im).astype(bf)
            v0=dNT(l3[0],T0); v2=dNT(l3[1],T2)
            return jnp.concatenate([v0+v2,v0-v2],axis=0)
        if t==1 and 'O' in OPT:
            X=jnp.where(leven,pltpu.roll(im,127,1),pltpu.roll(im,1,1))
            w1=dNT(l3[2],jnp.where(m03,re,X).astype(bf)); w3=dNT(l3[3],jnp.where(m03,X,re).astype(bf))
            a,b,c,d=w1[:56],w1[56:],w3[:56],w3[56:]
            r=math.sqrt(0.5)
            return jnp.concatenate([a+c,((a-b)-(c+d))*r,d-b,((c-d)-(a+b))*r],axis=0)
        V=jnp.concatenate([re,im],axis=1).astype(bf)
        return dNT(li[...],V)
    def build_b(j,r0):
        cs=slice(256*j,256*j+256)
        lo=slice(r0,r0+32); hi=slice(H+r0,H+r0+32)
        gl=wg[lo,cs].astype(f32); gh=wg[hi,cs].astype(f32); ul=wu[lo,cs].astype(f32); uh=wu[hi,cs].astype(f32)
        for i,v in enumerate((gl+uh,ul-uh,gh-gl,gl+ul,gh+uh)): bw[i,lo,cs]=v.astype(bf)
    def build_a(j0,r0):
        js=[j for j in (j0,j0+1) if j<7]
        cs=slice(128*j0,128*j0+128*len(js))
        lo=[wd[r0:r0+32,256*j:256*j+256].astype(f32) for j in js]
        hi=[wd[H+r0:H+r0+32,256*j:256*j+256].astype(f32) for j in js]
        def cat(l,odd): return jnp.concatenate([v[:,128*odd:128*odd+128] for v in l],axis=1)
        a11=cat(lo,0); a12=cat(lo,1); a21=cat(hi,0); a22=cat(hi,1)
        for i,v in enumerate((a11+a22,a21+a22,a11+a12,a21-a11,a12-a22)): aw[i,r0:r0+32,cs]=v.astype(bf)
    def bb(js): return [functools.partial(build_b,j,r0) for j in js for r0 in range(0,H,32)]
    def ba(): return [functools.partial(build_a,j0,r0) for j0 in range(0,7,2) for r0 in range(0,H,32)]
    gu_done=set()
    def wait_gu(js):
        for i,(a,b) in enumerate(GUC):
            if i not in gu_done and any(a<=j<b for j in js):
                gu_done.add(i)
                for d in d_gu[i]: d.wait()
    def mix(main,bg):
        steps=[]
        n=sum(m[1] for m in main); i=0; done=0
        for fn,cnt in main:
            g=fn()
            for _ in range(cnt):
                if g is not None: next(g)
                i+=1
                while done<len(bg) and done<len(bg)*i/n:
                    bg[done](); done+=1
            if g is not None:
                for _ in g: pass
        while done<len(bg): bg[done](); done+=1
    P=functools.partial
    def one(fn,*a):
        def g():
            fn(*a); yield
        return (g,1)
    with scope("P2F3E"): f3(0)
    with scope("P3AE"):
        d_nq[0].wait(); d_nq[1].wait(); d_w[0][0].wait(); d_w[0][1].wait()
        mix([one(stA,0,k1) for k1 in range(16)],[P(wt,0)]+(tasks2(zio,1,14,False) if TP[0]=='1' else [P(f3,1,[g]) for g in range(14)]))
    with scope("P4AO"):
        for c in (1,2): d_w[c][0].wait(); d_w[c][1].wait()
        mix([one(stA,1,k1) for k1 in range(8)],[P(wt,1),P(wt,2)])
        d_w[3][0].wait(); d_w[3][1].wait()
        mix([one(stA,1,k1) for k1 in range(8,16)],[P(wt,3)])
    with scope("P5BE"):
        for k1 in range(16): stB(0,k1)
    with scope("P6BO_F7E"):
        if BM=='0': wait_gu([0])
        mix([one(stB,1,k1) for k1 in range(16)],(tasks2(uio,0,16,True) if TP[1]=='1' else [P(f7g,0,g) for g in range(16)])+(bb([0]) if BM=='0' else []))
    def dve(ai): ve[:,128*ai:128*ai+128]=dinv(0,ai)
    with scope("P7DE_F7O"):
        d_li.wait(); d_l3.wait()
        if BM=='0': wait_gu([1,2])
        mix([one(dve,ai) for ai in range(16)],(tasks2(uio,1,16,True) if TP[2]=='1' else [P(f7g,1,g) for g in range(16)])+(bb([1,2]) if BM=='0' else []))
    outs=[]
    def prep1(c,q):
        ai=4*c+q; cs=slice(128*ai,128*ai+128); qs=slice(128*q,128*q+128)
        vo=dinv(1,ai); v0=ve[:,cs]
        x=xs[:,cs].astype(f32)
        h=jnp.concatenate([x[:H]+(v0+vo),x[H:]+(v0-vo)],axis=0).astype(bf)
        hb[c%3,:,qs]=h
        hf=h.astype(f32)
        m=jnp.sum(hf,axis=0,keepdims=True)*(1.0/D)
        hc=hf-m
        v=jnp.sum(hc*hc,axis=0,keepdims=True)*(1.0/D)
        lnf[:,qs]=hc*lax.rsqrt(v+1e-5)
    def prep1b(c,q):
        ai=4*c+q; cs=slice(128*ai,128*ai+128); qs=slice(128*q,128*q+128)
        vo=dinv(1,ai)
        s1=None; s2=None
        RB=int(PREP[1:])
        for r0 in range(0,H,RB):
            v0=ve[r0:r0+RB,cs]; v1=vo[r0:r0+RB]
            hl=(xs[r0:r0+RB,cs].astype(f32)+(v0+v1)).astype(bf); hh=(xs[H+r0:H+r0+RB,cs].astype(f32)+(v0-v1)).astype(bf)
            hb[c%3,r0:r0+RB,qs]=hl; hb[c%3,H+r0:H+r0+RB,qs]=hh
            a=hl.astype(f32); b=hh.astype(f32)
            t1=a+b; t2=a*a+b*b
            s1=t1 if s1 is None else s1+t1
            s2=t2 if s2 is None else s2+t2
        m=jnp.sum(s1,axis=0,keepdims=True)*(1.0/D)
        v=jnp.sum(s2,axis=0,keepdims=True)*(1.0/D)-m*m
        rr=lax.rsqrt(jnp.maximum(v,0.0)+1e-5)
        for r0 in range(0,D,RB):
            lnf[r0:r0+RB,qs]=(hb[c%3,r0:r0+RB,qs].astype(f32)-m)*rr
    def prep2(c,q):
        qa=slice(128*q,128*q+128); qb=slice(TH+128*q,TH+128*q+128)
        L11=lnf[0:H,qa]; L12=lnf[H:D,qa]; L21=lnf[0:H,qb]; L22=lnf[H:D,qb]
        for i,a in enumerate((L11+L22,L21+L22,L11,L22,L11+L12,L21-L11,L12-L22)):
            al[c%2,i,qa,:]=a.T.astype(bf)
    def prep_tasks(c):
        p1=prep1 if PREP=='0' else prep1b
        return [P(p1,c,0),P(p1,c,2),P(prep2,c,0),P(p1,c,1),P(p1,c,3),P(prep2,c,1)]
    def bsrc(i,cs):
        if i==1: return wg[0:H,cs]
        if i==4: return wu[H:D,cs]
        return bw[{0:0,2:1,3:2,5:3,6:4}[i],:,cs]
    keep=[]
    def gu(c,j):
        cs=slice(256*j,256*j+256); lo=slice(128*j,128*j+128)
        m=[None]*7
        for i in (1,4,2,0,3,6,5):
            m[i]=dNN(al[c%2,i],bsrc(i,cs)); yield
        ga=m[0]+m[3]-m[4]+m[6]; ua=m[2]+m[4]; gb=m[1]+m[3]; ub=m[0]-m[1]+m[2]+m[5]
        ha=ga*ua; hh=gb*ub
        alo=ha[:,0:128]; ahi=ha[:,128:256]; blo=hh[:,0:128]; bhi=hh[:,128:256]
        cb=(alo+bhi,alo,blo-bhi,ahi-alo,bhi,alo+blo,ahi+bhi)
        for p in range(3): bc[p,:,cs]=jnp.concatenate([cb[2*p],cb[2*p+1]],axis=1).astype(bf)
        bc[3,:,lo]=cb[6].astype(bf)
    def down(c):
        ds=[]
        def asrc(i):
            if i==2: return jnp.concatenate([wd[0:H,256*j:256*j+128] for j in range(7)],axis=1)
            if i==3: return jnp.concatenate([wd[H:D,256*j+128:256*j+256] for j in range(7)],axis=1)
            return aw[{0:0,1:1,4:2,5:3,6:4}[i]]
        def bsr(i):
            if i==6: return bc[3,:,0:FH]
            return jnp.concatenate([bc[i//2,:,256*j+128*(i%2):256*j+128*(i%2)+128] for j in range(7)],axis=1)
        def M(i): return dNT(asrc(i),bsr(i))
        def res(r0,c0): return hb[c%3,r0:r0+H,c0:c0+TH].astype(f32)
        def emit(r0,c0,v):
            ob[c,r0:r0+H,c0:c0+TH]=v.astype(bf)
            d=mk(ob.at[c,r0:r0+H,c0:c0+TH],o_h.at[r0:r0+H,c*T+c0:c*T+c0+TH]); d.start(); ds.append(d)
        m5=M(4); yield
        c11=res(0,0)-m5; c12=res(0,TH)+m5
        m3=M(2); yield
        emit(0,TH,c12+m3); c22=res(H,TH)+m3
        m2=M(1); yield
        c21=res(H,0)+m2; c22=c22-m2
        m4=M(3); yield
        emit(H,0,c21+m4); c11=c11+m4
        m1=M(0); yield
        c11=c11+m1; c22=c22+m1
        m7=M(6); yield
        emit(0,0,c11+m7)
        m6=M(5); yield
        emit(H,TH,c22+m6)
        outs.append(ds)
    with scope("P8prep0"):
        wait_gu([3,4])
        if BM=='1':
            wait_gu([0,1,2,5,6])
            for f in bb(range(7)): f()
        if BM in '34':
            wait_gu(range(7))
            for f in bb([0]): f()
        if BM=='2':
            wait_gu([0,1,2,5])
            for f in bb(range(6)): f()
        pt=prep_tasks(0); b34=bb([3,4]) if BM=='0' else []
        if BM=='4': pass
        for i,t_ in enumerate(pt):
            t_()
            for f in b34[i*len(b34)//len(pt):(i+1)*len(b34)//len(pt)]: f()
    with scope("P9back0"):
        if BM=='0':
            wait_gu([5,6]); d_wd.wait()
            mix([(P(gu,0,j),7) for j in range(7)],bb([5,6])+prep_tasks(1)+ba())
        elif BM=='3':
            d_wd.wait()
            mix([(P(gu,0,j),7) for j in range(7)],bb(range(1,7))+prep_tasks(1)+ba())
        elif BM=='4':
            d_wd.wait()
            mix([(P(gu,0,j),7) for j in range(7)],bb(range(1,7))+prep_tasks(1))
        elif BM=='2':
            d_wd.wait()
            for f in ba(): f()
            wait_gu([6])
            mix([(P(gu,0,j),7) for j in range(7)],bb([6])+prep_tasks(1))
        else:
            d_wd.wait()
            for f in ba(): f()
            mix([(P(gu,0,j),7) for j in range(7)],prep_tasks(1))
        if BM=='4':
            for f in ba(): f()
        mix([(P(down,0),7)],[])
    for c in range(1,4):
        with scope(f"P9back{c}"):
            mix([(P(gu,c,j),7) for j in range(7)],prep_tasks(c+1) if c<3 else [])
            mix([(P(down,c),7)],[])
    with scope("PZwaitout"):
        for ds in outs:
            for d in ds: d.wait()

@jax.jit
def pallas_sequential_preLN__spectral_gfnet__glu_gated_bilinear__prompt_kernel(A_x,A_w_r,A_w_i,B_x,B_w_gate,B_w_up,B_w_down):
    xT=A_x.reshape(S,D).T; wrT=A_w_r.T; wiT=A_w_i.T; wdT=B_w_down.T
    Ld=jnp.asarray(d_fwd2().astype(BF)); Li=jnp.asarray(d_inv2()[1].astype(BF)); Le=jnp.asarray(d_fwd3()[0].astype(BF)); L3=jnp.asarray(d_inv3()[0:2].astype(BF))
    anyspec=pl.BlockSpec(memory_space=pltpu.HBM)
    out=pl.pallas_call(kernel,
        out_shape=jax.ShapeDtypeStruct((D,S),bf),
        in_specs=[anyspec]*10,out_specs=anyspec,
        scratch_shapes=[pltpu.VMEM((D,S),bf),pltpu.VMEM((2,224,S),bf),pltpu.VMEM((2,1,S),bf),
            pltpu.VMEM((D,F),bf),pltpu.VMEM((D,F),bf),pltpu.VMEM((D,F),bf),
            pltpu.VMEM((2,224,H),bf),pltpu.VMEM((H,256),bf),
            pltpu.VMEM((16,192,128),u32) if 'u' in OPT else pltpu.VMEM((16,384,128),bf),
            pltpu.VMEM((2,2,16,112,128),f32),pltpu.VMEM((2,2,16,128,128),f32),(pltpu.VMEM((2,2,17*128,128),f32) if 'w' in OPT else pltpu.VMEM((2,17*128,128),u32)),pltpu.VMEM((2,2,S,128),f32),
            pltpu.VMEM((H,S),f32),pltpu.VMEM((D,T),f32),
            pltpu.VMEM((2,7,TH,H),bf),pltpu.VMEM((3,D,T),bf),pltpu.VMEM((4,D,T),bf),
            pltpu.VMEM((5,H,F),bf),pltpu.VMEM((5,H,FH),bf),pltpu.VMEM((4,TH,F),bf),
            pltpu.VMEM((2,112,112),bf),pltpu.VMEM((2,112,128),bf),
            pltpu.SemaphoreType.DMA((80,))],
        compiler_params=pltpu.CompilerParams(vmem_limit_bytes=100*1024*1024),
    )(xT,wrT,wiT,B_w_gate,B_w_up,wdT,Ld,Li,Le,L3)
    return out.T.reshape(1,S,D)
```

```python
import functools
import math

import jax
import jax.numpy as jnp
import ml_dtypes
import numpy as np
from jax import lax
import jax.experimental.pallas as pl
import jax.experimental.pallas.tpu as pltpu

S, D, F = 2048, 448, 1792
H = D // 2
FH = F // 2
T = 512
TH = T // 2
EPS = 1e-5

bf = jnp.bfloat16
f32 = jnp.float32
u32 = jnp.uint32
P = functools.partial

_NT = (((1,), (1,)), ((), ()))
_TN = (((0,), (0,)), ((), ()))


def d_nn(a, b):
    return jnp.dot(a, b, preferred_element_type=f32)


def d_nt(a, b):
    return lax.dot_general(a, b, _NT, preferred_element_type=f32)


def d_tn(a, b):
    return lax.dot_general(a, b, _TN, preferred_element_type=f32)


def _cos_sin(num, den):
    a = 2 * np.pi * np.mod(num, den) / den
    c, s = np.cos(a), np.sin(a)
    return np.where(np.abs(c) < 1e-12, 0, c), np.where(np.abs(s) < 1e-12, 0, s)


def _inverse_d_matrices():
    k_even = 2 * np.arange(112)
    k_even[0] = H
    k_odd = 2 * np.arange(112) + 1
    scale = 1.0 / (D * S)
    odd = np.zeros((H, 256))
    c, s = _cos_sin(np.arange(H)[:, None] * k_odd[None, :], D)
    odd[:, :112] = 2 * scale * c
    odd[:, 128:240] = -2 * scale * s
    even = np.zeros((2, 112, 128))
    for j, k in enumerate((k_even[0::2], k_even[1::2])):
        w = np.where(k == H, 1.0, 2.0) * scale
        c, s = _cos_sin(np.arange(112)[:, None] * k[None, :], D)
        even[j, :, 0:112:2] = c * w
        even[j, :, 1:112:2] = -s * w
    return odd.astype(ml_dtypes.bfloat16), even.astype(ml_dtypes.bfloat16)


def _cadd(a, b):
    return a[0] + b[0], a[1] + b[1]


def _csub(a, b):
    return a[0] - b[0], a[1] - b[1]


def _fft4(x, inv):
    t0, t1 = _cadd(x[0], x[2]), _csub(x[0], x[2])
    t2, t3 = _cadd(x[1], x[3]), _csub(x[1], x[3])
    mi = (t1[0] + t3[1], t1[1] - t3[0])
    pi = (t1[0] - t3[1], t1[1] + t3[0])
    return [_cadd(t0, t2), pi if inv else mi, _csub(t0, t2), mi if inv else pi]


def _tw16(x, e, inv):
    a, b = x
    if e == 0:
        return x
    if e == 4:
        return (-b, a) if inv else (b, -a)
    c = math.cos(2 * math.pi * e / 16)
    s = math.sin(2 * math.pi * e / 16) * (1 if inv else -1)
    if e in (2, 6):
        r = abs(c)
        if c > 0 and s > 0:
            return (a - b) * r, (a + b) * r
        if c > 0 and s < 0:
            return (a + b) * r, (b - a) * r
        if c < 0 and s > 0:
            return (a + b) * (-r), (a - b) * r
        return (b - a) * r, (a + b) * (-r)
    return a * c - b * s, b * c + a * s


def _fft16(x, inv):
    t = [None] * 16
    for a0 in range(4):
        y = _fft4([x[4 * a1 + a0] for a1 in range(4)], inv)
        for k0 in range(4):
            t[4 * a0 + k0] = _tw16(y[k0], a0 * k0, inv)
    out = [None] * 16
    for k0 in range(4):
        y = _fft4([t[4 * a0 + k0] for a0 in range(4)], inv)
        for k in range(4):
            out[k0 + 4 * k] = y[k]
    return out


def _interleave(main, side):
    n = sum(cnt for _, cnt in main)
    i = done = 0
    for fn, cnt in main:
        g = fn()
        for _ in range(cnt):
            next(g)
            i += 1
            while done < len(side) and done < len(side) * i / n:
                side[done]()
                done += 1
        for _ in g:
            pass
    while done < len(side):
        side[done]()
        done += 1


def _step(fn, *args):
    def gen():
        fn(*args)
        yield
    return gen, 1


def _kernel(x_h, wr_h, wi_h, wg_h, wu_h, wd_h, lo_h, le_h, o_h,
            xs, wraw, nyq, wg, wu, wd, ldf, lio, lie, mf, z_s, y_s, wt_s, u_s, ve, lnf,
            al, hb, ob, bw, aw, bc, sem):
    sem_ids = iter(range(48))

    def dma(src, dst):
        return pltpu.make_async_copy(src, dst, sem.at[next(sem_ids)])

    d_x = [dma(x_h.at[:, 512 * c:512 * c + 512], xs.at[:, 512 * c:512 * c + 512]) for c in range(4)]
    d_nq = [dma(wr_h.at[H:H + 1, :], nyq.at[0]), dma(wi_h.at[H:H + 1, :], nyq.at[1])]
    d_w = [[dma(w.at[0:H, 512 * c:512 * c + 512], wraw.at[i, :, 512 * c:512 * c + 512])
            for i, w in enumerate((wr_h, wi_h))] for c in range(4)]
    d_li = [dma(lo_h, lio), dma(le_h, lie)]
    d_gu = [dma(wg_h, wg), dma(wu_h, wu)]
    d_wd = dma(wd_h, wd)
    for d in d_x + d_nq + [d for ds in d_w for d in ds] + d_li + d_gu + [d_wd]:
        d.start()

    r = lax.broadcasted_iota(jnp.int32, (128, 128), 0)
    c_ = lax.broadcasted_iota(jnp.int32, (128, 128), 1)
    ang = ((r * c_) & 127).astype(f32) * (2 * math.pi / 128)
    c0, s0 = jnp.cos(ang), -jnp.sin(ang)
    r2 = lax.broadcasted_iota(jnp.int32, (16, 128), 0)
    c2 = lax.broadcasted_iota(jnp.int32, (16, 128), 1)
    a2 = (r2 * c2).astype(f32) * (2 * math.pi / S)
    tc, ts = jnp.cos(a2), -jnp.sin(a2)
    for k1 in range(16):
        if k1 == 0:
            cm, sm = c0, s0
        else:
            a, b = tc[k1:k1 + 1, :], ts[k1:k1 + 1, :]
            cm, sm = c0 * a - s0 * b, c0 * b + s0 * a
        for j, m in enumerate((cm, sm - cm, cm + sm)):
            mf[k1, 128 * j:128 * j + 128, :] = m.astype(bf)

    def cs_d(n):
        n = n.astype(f32)
        n = n - jnp.floor(n * (1.0 / D)) * D
        a_ = n * (2 * math.pi / D)
        return jnp.cos(a_), -jnp.sin(a_)

    stc, sts = cs_d(16 * lax.broadcasted_iota(jnp.int32, (16, H), 0)
                    * lax.broadcasted_iota(jnp.int32, (16, H), 1))
    s8 = lax.broadcasted_iota(jnp.int32, (8, H), 0)
    d8 = lax.broadcasted_iota(jnp.int32, (8, H), 1)
    for t in range(2):
        bc_, bs_ = cs_d((2 * s8 + t) * d8)
        cr, sr = [], []
        for g in range(14):
            if g == 0:
                c1, s1 = bc_, bs_
            else:
                sc, ss = stc[g:g + 1, :], sts[g:g + 1, :]
                c1, s1 = bc_ * sc - bs_ * ss, bc_ * ss + bs_ * sc
            if g == 0 and t == 0:
                c1 = jnp.where(s8 == 0, (1 - 2 * (d8 & 1)).astype(f32), c1)
                s1 = jnp.where(s8 == 0, 0.0, s1)
            cr.append(c1)
            sr.append(s1)
        ldf[t, 0:112, :] = jnp.concatenate(cr, axis=0).astype(bf)
        ldf[t, 112:H, :] = jnp.concatenate(sr, axis=0).astype(bf)

    def d_forward(ai):
        cs = slice(128 * ai, 128 * ai + 128)
        lo, hi = xs[0:H, cs].astype(f32), xs[H:D, cs].astype(f32)
        o = lo - hi
        obf = o.astype(bf)
        e = lo + hi
        so = jnp.sum(o * o, axis=0, keepdims=True)
        ec = e - jnp.sum(e, axis=0, keepdims=True) * (1.0 / H)
        ebf = ec.astype(bf)
        ss = so + jnp.sum(ec * ec, axis=0, keepdims=True)
        rr = lax.rsqrt(ss * (0.5 / D) + EPS)
        for t, v in enumerate((ebf, obf)):
            z = d_nn(ldf[t], v) * rr
            z_s[t, 0, ai] = z[:112]
            z_s[t, 1, ai] = z[112:]

    for c in range(4):
        d_x[c].wait()
        for ai in range(4 * c, 4 * c + 4):
            d_forward(ai)

    def radix16_fwd(t, groups):
        for g in groups:
            rows = slice(8 * g, 8 * g + 8)
            y = _fft16([(z_s[t, 0, a, rows, :], z_s[t, 1, a, rows, :]) for a in range(16)], False)
            for k in range(16):
                z_s[t, 0, k, rows, :] = y[k][0]
                z_s[t, 1, k, rows, :] = y[k][1]

    def radix16_inv(t, g):
        def rows(a):
            return slice(128 * a + 8 * g, 128 * a + 8 * g + 8)
        y = _fft16([(u_s[0, t, rows(k), :], u_s[1, t, rows(k), :]) for k in range(16)], True)
        for a in range(16):
            u_s[0, t, rows(a), :] = y[a][0]
            u_s[1, t, rows(a), :] = y[a][1]

    def filter_t(c):
        for ri in range(2):
            for p in range(4 * c, 4 * c + 4):
                cs = slice(128 * p, 128 * p + 128)
                w = pltpu.bitcast(wraw[ri, :, cs], u32)
                nq = lax.shift_right_logical(
                    pltpu.bitcast(nyq[ri, :, cs].astype(f32), u32), jnp.uint32(16))
                row0 = lax.broadcasted_iota(jnp.int32, (8, 128), 0) == 0
                first = jnp.where(row0, (w[0:8] & jnp.uint32(0xFFFF0000)) | nq, w[0:8])
                tt = jnp.concatenate([first, w[8:112], jnp.zeros((16, 128), u32)], axis=0).T
                for g in range(16):
                    r_ = 17 * (8 * p + g // 2) + 8 * (g % 2)
                    wt_s[ri, r_:r_ + 8, :] = tt[8 * g:8 * g + 8]

    zpad = jnp.zeros((16, 128), f32)

    def pad_bf(v):
        return jnp.concatenate([v, zpad], axis=0).astype(bf)

    def mat(k1, j):
        return mf[k1, 128 * j:128 * j + 128, :]

    def s_forward(t, k1):
        a, b = z_s[t, 0, k1], z_s[t, 1, k1]
        m1 = d_nt(mat(k1, 0), pad_bf(a + b))
        m2 = d_nt(mat(k1, 1), pad_bf(a))
        m3 = d_nt(mat(k1, 2), pad_bf(b))
        y_s[0, t, k1] = m1 - m3
        y_s[1, t, k1] = m1 + m2

    def s_inverse(t, k1):
        def half(v):
            if t == 0:
                return pltpu.bitcast(v << jnp.uint32(16), f32)
            return pltpu.bitcast(v & jnp.uint32(0xFFFF0000), f32)
        wr = half(wt_s[0, pl.ds(k1, 128, stride=17), :])
        wi = half(wt_s[1, pl.ds(k1, 128, stride=17), :])
        yr0, yi0 = y_s[0, t, k1], y_s[1, t, k1]
        yr, yi = yr0 * wr - yi0 * wi, yr0 * wi + yi0 * wr
        m1 = d_tn(mat(k1, 0), (yr + yi).astype(bf))
        m2 = d_tn(mat(k1, 1), yi.astype(bf))
        m3 = d_tn(mat(k1, 2), yr.astype(bf))
        u_s[0, t, 128 * k1:128 * k1 + 128, :] = m1 + m2
        u_s[1, t, 128 * k1:128 * k1 + 128, :] = m1 - m3

    lane_even = (lax.broadcasted_iota(jnp.int32, (128, 128), 1) & 1) == 0

    def d_inverse_even(ai):
        rs = slice(128 * ai, 128 * ai + 128)
        re, im = u_s[0, 0, rs, :], u_s[1, 0, rs, :]
        t0 = jnp.where(lane_even, re, pltpu.roll(im, 1, 1)).astype(bf)
        t2 = jnp.where(lane_even, pltpu.roll(re, 127, 1), im).astype(bf)
        v0, v2 = d_nt(lie[0], t0), d_nt(lie[1], t2)
        ve[:, rs] = jnp.concatenate([v0 + v2, v0 - v2], axis=0)

    def d_inverse_odd(ai):
        rs = slice(128 * ai, 128 * ai + 128)
        v = jnp.concatenate([u_s[0, 1, rs, :], u_s[1, 1, rs, :]], axis=1).astype(bf)
        return d_nt(lio[...], v)

    def build_b(j, r0):
        cs = slice(256 * j, 256 * j + 256)
        lo, hi = slice(r0, r0 + 32), slice(H + r0, H + r0 + 32)
        gl, gh = wg[lo, cs].astype(f32), wg[hi, cs].astype(f32)
        ul, uh = wu[lo, cs].astype(f32), wu[hi, cs].astype(f32)
        for i, v in enumerate((gl + uh, ul - uh, gh - gl, gl + ul, gh + uh)):
            bw[i, lo, cs] = v.astype(bf)

    def build_a(j0, r0):
        js = [j for j in (j0, j0 + 1) if j < 7]
        cs = slice(128 * j0, 128 * j0 + 128 * len(js))
        lo = [wd[r0:r0 + 32, 256 * j:256 * j + 256].astype(f32) for j in js]
        hi = [wd[H + r0:H + r0 + 32, 256 * j:256 * j + 256].astype(f32) for j in js]

        def cat(vs, odd):
            return jnp.concatenate([v[:, 128 * odd:128 * odd + 128] for v in vs], axis=1)
        a11, a12, a21, a22 = cat(lo, 0), cat(lo, 1), cat(hi, 0), cat(hi, 1)
        for i, v in enumerate((a11 + a22, a21 + a22, a11 + a12, a21 - a11, a12 - a22)):
            aw[i, r0:r0 + 32, cs] = v.astype(bf)

    def prep_norm(c, q):
        ai = 4 * c + q
        cs, qs = slice(128 * ai, 128 * ai + 128), slice(128 * q, 128 * q + 128)
        vo = d_inverse_odd(ai)
        s1 = s2 = None
        for r0 in range(0, H, 32):
            v0, v1 = ve[r0:r0 + 32, cs], vo[r0:r0 + 32]
            hl = (xs[r0:r0 + 32, cs].astype(f32) + (v0 + v1)).astype(bf)
            hh = (xs[H + r0:H + r0 + 32, cs].astype(f32) + (v0 - v1)).astype(bf)
            hb[c % 3, r0:r0 + 32, qs] = hl
            hb[c % 3, H + r0:H + r0 + 32, qs] = hh
            a, b = hl.astype(f32), hh.astype(f32)
            t1, t2 = a + b, a * a + b * b
            s1 = t1 if s1 is None else s1 + t1
            s2 = t2 if s2 is None else s2 + t2
        m = jnp.sum(s1, axis=0, keepdims=True) * (1.0 / D)
        var = jnp.sum(s2, axis=0, keepdims=True) * (1.0 / D) - m * m
        rr = lax.rsqrt(jnp.maximum(var, 0.0) + EPS)
        for r0 in range(0, D, 32):
            lnf[r0:r0 + 32, qs] = (hb[c % 3, r0:r0 + 32, qs].astype(f32) - m) * rr

    def prep_sums(c, q):
        qa, qb = slice(128 * q, 128 * q + 128), slice(TH + 128 * q, TH + 128 * q + 128)
        l11, l12, l21, l22 = lnf[0:H, qa], lnf[H:D, qa], lnf[0:H, qb], lnf[H:D, qb]
        for i, a in enumerate((l11 + l22, l21 + l22, l11, l22, l11 + l12, l21 - l11, l12 - l22)):
            al[c % 2, i, qa, :] = a.T.astype(bf)

    def prep_tasks(c):
        out = []
        for q in range(2):
            out += [P(prep_norm, c, q), P(prep_norm, c, 2 + q), P(prep_sums, c, q)]
        return out

    def gate_up(c, j):
        cs, lo = slice(256 * j, 256 * j + 256), slice(128 * j, 128 * j + 128)

        def rhs(i):
            if i == 1:
                return wg[0:H, cs]
            if i == 4:
                return wu[H:D, cs]
            return bw[{0: 0, 2: 1, 3: 2, 5: 3, 6: 4}[i], :, cs]
        m = [None] * 7
        for i in (1, 4, 2, 0, 3, 6, 5):
            m[i] = d_nn(al[c % 2, i], rhs(i))
            yield
        ha = (m[0] + m[3] - m[4] + m[6]) * (m[2] + m[4])
        hh = (m[1] + m[3]) * (m[0] - m[1] + m[2] + m[5])
        alo, ahi, blo, bhi = ha[:, 0:128], ha[:, 128:256], hh[:, 0:128], hh[:, 128:256]
        cb = (alo + bhi, alo, blo - bhi, ahi - alo, bhi, alo + blo, ahi + bhi)
        for p in range(3):
            bc[p, :, cs] = jnp.concatenate([cb[2 * p], cb[2 * p + 1]], axis=1).astype(bf)
        bc[3, :, lo] = cb[6].astype(bf)

    outs = []

    def down(c):
        def lhs(i):
            if i == 2:
                return jnp.concatenate([wd[0:H, 256 * j:256 * j + 128] for j in range(7)], axis=1)
            if i == 3:
                return jnp.concatenate([wd[H:D, 256 * j + 128:256 * j + 256] for j in range(7)], axis=1)
            return aw[{0: 0, 1: 1, 4: 2, 5: 3, 6: 4}[i]]

        def rhs(i):
            if i == 6:
                return bc[3, :, 0:FH]
            off = 128 * (i % 2)
            return jnp.concatenate(
                [bc[i // 2, :, 256 * j + off:256 * j + off + 128] for j in range(7)], axis=1)

        def prod(i):
            return d_nt(lhs(i), rhs(i))

        def res(r0, c0):
            return hb[c % 3, r0:r0 + H, c0:c0 + TH].astype(f32)

        def emit(r0, c0, v):
            cols = slice(c * T + c0, c * T + c0 + TH)
            ob[r0:r0 + H, cols] = v.astype(bf)
            d = dma(ob.at[r0:r0 + H, cols], o_h.at[r0:r0 + H, cols])
            d.start()
            outs.append(d)

        m5 = prod(4)
        yield
        c11, c12 = res(0, 0) - m5, res(0, TH) + m5
        m3 = prod(2)
        yield
        emit(0, TH, c12 + m3)
        c22 = res(H, TH) + m3
        m2 = prod(1)
        yield
        c21, c22 = res(H, 0) + m2, c22 - m2
        m4 = prod(3)
        yield
        emit(H, 0, c21 + m4)
        c11 = c11 + m4
        m1 = prod(0)
        yield
        c11, c22 = c11 + m1, c22 + m1
        m7 = prod(6)
        yield
        emit(0, 0, c11 + m7)
        m6 = prod(5)
        yield
        emit(H, TH, c22 + m6)

    radix16_fwd(0, range(14))

    for d in d_nq + d_w[0]:
        d.wait()
    _interleave([_step(s_forward, 0, k1) for k1 in range(16)],
                [P(filter_t, 0)] + [P(radix16_fwd, 1, [g]) for g in range(14)])

    for d in d_w[1] + d_w[2]:
        d.wait()
    _interleave([_step(s_forward, 1, k1) for k1 in range(8)], [P(filter_t, 1), P(filter_t, 2)])
    for d in d_w[3]:
        d.wait()
    _interleave([_step(s_forward, 1, k1) for k1 in range(8, 16)], [P(filter_t, 3)])

    for k1 in range(16):
        s_inverse(0, k1)
    _interleave([_step(s_inverse, 1, k1) for k1 in range(16)],
                [P(radix16_inv, 0, g) for g in range(16)])

    for d in d_li:
        d.wait()
    _interleave([_step(d_inverse_even, ai) for ai in range(16)],
                [P(radix16_inv, 1, g) for g in range(16)])

    for d in d_gu:
        d.wait()
    for j in range(7):
        for r0 in range(0, H, 32):
            build_b(j, r0)
    for task in prep_tasks(0):
        task()

    for c in range(4):
        if c == 0:
            d_wd.wait()
            for j0 in range(0, 7, 2):
                for r0 in range(0, H, 32):
                    build_a(j0, r0)
        _interleave([(P(gate_up, c, j), 7) for j in range(7)], prep_tasks(c + 1) if c < 3 else [])
        _interleave([(P(down, c), 7)], [])

    for d in outs:
        d.wait()


@jax.jit
def pallas_sequential_preLN__spectral_gfnet__glu_gated_bilinear__prompt_kernel(
    A_x: jax.Array,
    A_w_r: jax.Array,
    A_w_i: jax.Array,
    B_x: jax.Array,
    B_w_gate: jax.Array,
    B_w_up: jax.Array,
    B_w_down: jax.Array,
):
    del B_x
    li_odd, li_even = _inverse_d_matrices()
    hbm = pl.BlockSpec(memory_space=pltpu.HBM)
    vmem = pltpu.VMEM
    out = pl.pallas_call(
        _kernel,
        out_shape=jax.ShapeDtypeStruct((D, S), bf),
        in_specs=[hbm] * 8,
        out_specs=hbm,
        scratch_shapes=[
            vmem((D, S), bf),
            vmem((2, H, S), bf),
            vmem((2, 1, S), bf),
            vmem((D, F), bf),
            vmem((D, F), bf),
            vmem((D, F), bf),
            vmem((2, H, H), bf),
            vmem((H, 256), bf),
            vmem((2, 112, 128), bf),
            vmem((16, 384, 128), bf),
            vmem((2, 2, 16, 112, 128), f32),
            vmem((2, 2, 16, 128, 128), f32),
            vmem((2, 17 * 128, 128), u32),
            vmem((2, 2, S, 128), f32),
            vmem((H, S), f32),
            vmem((D, T), f32),
            vmem((2, 7, TH, H), bf),
            vmem((3, D, T), bf),
            vmem((D, S), bf),
            vmem((5, H, F), bf),
            vmem((5, H, FH), bf),
            vmem((4, TH, F), bf),
            pltpu.SemaphoreType.DMA((48,)),
        ],
        compiler_params=pltpu.CompilerParams(vmem_limit_bytes=100 * 1024 * 1024),
    )(A_x.reshape(S, D).T, A_w_r.T, A_w_i.T, B_w_gate, B_w_up, B_w_down.T, li_odd, li_even)
    return out.T.reshape(1, S, D)
```

```python
import functools
import math

import jax
import jax.numpy as jnp
import ml_dtypes
import numpy as np
from jax import lax
import jax.experimental.pallas as pl
import jax.experimental.pallas.tpu as pltpu

S, D, F = 2048, 448, 1792
H = D // 2
FH = F // 2
T = 512
TH = T // 2
EPS = 1e-5

bf = jnp.bfloat16
f32 = jnp.float32
u32 = jnp.uint32
P = functools.partial

_NT = (((1,), (1,)), ((), ()))
_TN = (((0,), (0,)), ((), ()))


def d_nn(a, b):
    return jnp.dot(a, b, preferred_element_type=f32)


def d_nt(a, b):
    return lax.dot_general(a, b, _NT, preferred_element_type=f32)


def d_tn(a, b):
    return lax.dot_general(a, b, _TN, preferred_element_type=f32)


def _cos_sin(num, den):
    a = 2 * np.pi * np.mod(num, den) / den
    c, s = np.cos(a), np.sin(a)
    return np.where(np.abs(c) < 1e-12, 0, c), np.where(np.abs(s) < 1e-12, 0, s)


def _inverse_d_matrices():
    k_even = 2 * np.arange(112)
    k_even[0] = H
    k_odd = 2 * np.arange(112) + 1
    scale = 1.0 / (D * S)
    odd = np.zeros((H, 256))
    c, s = _cos_sin(np.arange(H)[:, None] * k_odd[None, :], D)
    odd[:, :112] = 2 * scale * c
    odd[:, 128:240] = -2 * scale * s
    even = np.zeros((2, 112, 128))
    for j, k in enumerate((k_even[0::2], k_even[1::2])):
        w = np.where(k == H, 1.0, 2.0) * scale
        c, s = _cos_sin(np.arange(112)[:, None] * k[None, :], D)
        even[j, :, 0:112:2] = c * w
        even[j, :, 1:112:2] = -s * w
    return odd.astype(ml_dtypes.bfloat16), even.astype(ml_dtypes.bfloat16)


def _cadd(a, b):
    return a[0] + b[0], a[1] + b[1]


def _csub(a, b):
    return a[0] - b[0], a[1] - b[1]


def _fft4(x, inv):
    t0, t1 = _cadd(x[0], x[2]), _csub(x[0], x[2])
    t2, t3 = _cadd(x[1], x[3]), _csub(x[1], x[3])
    mi = (t1[0] + t3[1], t1[1] - t3[0])
    pi = (t1[0] - t3[1], t1[1] + t3[0])
    return [_cadd(t0, t2), pi if inv else mi, _csub(t0, t2), mi if inv else pi]


def _tw16(x, e, inv):
    a, b = x
    if e == 0:
        return x
    if e == 4:
        return (-b, a) if inv else (b, -a)
    c = math.cos(2 * math.pi * e / 16)
    s = math.sin(2 * math.pi * e / 16) * (1 if inv else -1)
    if e in (2, 6):
        r = abs(c)
        if c > 0 and s > 0:
            return (a - b) * r, (a + b) * r
        if c > 0 and s < 0:
            return (a + b) * r, (b - a) * r
        if c < 0 and s > 0:
            return (a + b) * (-r), (a - b) * r
        return (b - a) * r, (a + b) * (-r)
    return a * c - b * s, b * c + a * s


def _fft16(x, inv):
    t = [None] * 16
    for a0 in range(4):
        y = _fft4([x[4 * a1 + a0] for a1 in range(4)], inv)
        for k0 in range(4):
            t[4 * a0 + k0] = _tw16(y[k0], a0 * k0, inv)
    out = [None] * 16
    for k0 in range(4):
        y = _fft4([t[4 * a0 + k0] for a0 in range(4)], inv)
        for k in range(4):
            out[k0 + 4 * k] = y[k]
    return out


def _interleave(main, side):
    n = sum(cnt for _, cnt in main)
    i = done = 0
    for fn, cnt in main:
        g = fn()
        for _ in range(cnt):
            next(g)
            i += 1
            while done < len(side) and done < len(side) * i / n:
                side[done]()
                done += 1
        for _ in g:
            pass
    while done < len(side):
        side[done]()
        done += 1


def _step(fn, *args):
    def gen():
        fn(*args)
        yield
    return gen, 1


def _kernel(x_h, wr_h, wi_h, wg_h, wu_h, wd_h, lo_h, le_h, o_h,
            xs, wraw, nyq, wg, wu, wd, ldf, lio, lie, mf, z_s, y_s, wt_s, u_s, ve, lnf,
            al, hb, ob, bw, aw, bc, sem):
    sem_ids = iter(range(48))

    def dma(src, dst):
        return pltpu.make_async_copy(src, dst, sem.at[next(sem_ids)])

    d_x = [dma(x_h.at[:, 512 * c:512 * c + 512], xs.at[:, 512 * c:512 * c + 512]) for c in range(4)]
    d_nq = [dma(wr_h.at[H:H + 1, :], nyq.at[0]), dma(wi_h.at[H:H + 1, :], nyq.at[1])]
    d_w = [[dma(w.at[0:H, 512 * c:512 * c + 512], wraw.at[i, :, 512 * c:512 * c + 512])
            for i, w in enumerate((wr_h, wi_h))] for c in range(4)]
    d_li = [dma(lo_h, lio), dma(le_h, lie)]
    d_gu = [dma(wg_h, wg), dma(wu_h, wu)]
    d_wd = dma(wd_h, wd)
    for d in d_x + d_nq + [d for ds in d_w for d in ds] + d_li + d_gu + [d_wd]:
        d.start()

    r = lax.broadcasted_iota(jnp.int32, (128, 128), 0)
    c_ = lax.broadcasted_iota(jnp.int32, (128, 128), 1)
    ang = ((r * c_) & 127).astype(f32) * (2 * math.pi / 128)
    c0, s0 = jnp.cos(ang), -jnp.sin(ang)
    r2 = lax.broadcasted_iota(jnp.int32, (16, 128), 0)
    c2 = lax.broadcasted_iota(jnp.int32, (16, 128), 1)
    a2 = (r2 * c2).astype(f32) * (2 * math.pi / S)
    tc, ts = jnp.cos(a2), -jnp.sin(a2)
    for k1 in range(16):
        if k1 == 0:
            cm, sm = c0, s0
        else:
            a, b = tc[k1:k1 + 1, :], ts[k1:k1 + 1, :]
            cm, sm = c0 * a - s0 * b, c0 * b + s0 * a
        for j, m in enumerate((cm, sm - cm, cm + sm)):
            mf[k1, 128 * j:128 * j + 128, :] = m.astype(bf)

    def cs_d(n):
        n = n.astype(f32)
        n = n - jnp.floor(n * (1.0 / D)) * D
        a_ = n * (2 * math.pi / D)
        return jnp.cos(a_), -jnp.sin(a_)

    stc, sts = cs_d(16 * lax.broadcasted_iota(jnp.int32, (16, H), 0)
                    * lax.broadcasted_iota(jnp.int32, (16, H), 1))
    s8 = lax.broadcasted_iota(jnp.int32, (8, H), 0)
    d8 = lax.broadcasted_iota(jnp.int32, (8, H), 1)
    for t in range(2):
        bc_, bs_ = cs_d((2 * s8 + t) * d8)
        cr, sr = [], []
        for g in range(14):
            if g == 0:
                c1, s1 = bc_, bs_
            else:
                sc, ss = stc[g:g + 1, :], sts[g:g + 1, :]
                c1, s1 = bc_ * sc - bs_ * ss, bc_ * ss + bs_ * sc
            if g == 0 and t == 0:
                c1 = jnp.where(s8 == 0, (1 - 2 * (d8 & 1)).astype(f32), c1)
                s1 = jnp.where(s8 == 0, 0.0, s1)
            cr.append(c1)
            sr.append(s1)
        ldf[t, 0:112, :] = jnp.concatenate(cr, axis=0).astype(bf)
        ldf[t, 112:H, :] = jnp.concatenate(sr, axis=0).astype(bf)

    def d_forward(ai):
        cs = slice(128 * ai, 128 * ai + 128)
        lo, hi = xs[0:H, cs].astype(f32), xs[H:D, cs].astype(f32)
        o = lo - hi
        obf = o.astype(bf)
        e = lo + hi
        so = jnp.sum(o * o, axis=0, keepdims=True)
        ec = e - jnp.sum(e, axis=0, keepdims=True) * (1.0 / H)
        ebf = ec.astype(bf)
        ss = so + jnp.sum(ec * ec, axis=0, keepdims=True)
        rr = lax.rsqrt(ss * (0.5 / D) + EPS)
        for t, v in enumerate((ebf, obf)):
            z = d_nn(ldf[t], v) * rr
            z_s[t, 0, ai] = z[:112]
            z_s[t, 1, ai] = z[112:]

    for c in range(4):
        d_x[c].wait()
        for ai in range(4 * c, 4 * c + 4):
            d_forward(ai)

    def radix16_fwd(t, groups):
        for g in groups:
            rows = slice(8 * g, 8 * g + 8)
            y = _fft16([(z_s[t, 0, a, rows, :], z_s[t, 1, a, rows, :]) for a in range(16)], False)
            for k in range(16):
                z_s[t, 0, k, rows, :] = y[k][0]
                z_s[t, 1, k, rows, :] = y[k][1]

    def radix16_inv(t, g):
        def rows(a):
            return slice(128 * a + 8 * g, 128 * a + 8 * g + 8)
        y = _fft16([(u_s[0, t, rows(k), :], u_s[1, t, rows(k), :]) for k in range(16)], True)
        for a in range(16):
            u_s[0, t, rows(a), :] = y[a][0]
            u_s[1, t, rows(a), :] = y[a][1]

    def filter_t(c):
        for ri in range(2):
            for p in range(4 * c, 4 * c + 4):
                cs = slice(128 * p, 128 * p + 128)
                w = pltpu.bitcast(wraw[ri, :, cs], u32)
                nq = lax.shift_right_logical(
                    pltpu.bitcast(nyq[ri, :, cs].astype(f32), u32), np.uint32(16))
                row0 = lax.broadcasted_iota(jnp.int32, (8, 128), 0) == 0
                first = jnp.where(row0, (w[0:8] & np.uint32(0xFFFF0000)) | nq, w[0:8])
                tt = jnp.concatenate([first, w[8:112], jnp.zeros((16, 128), u32)], axis=0).T
                for g in range(16):
                    r_ = 17 * (8 * p + g // 2) + 8 * (g % 2)
                    wt_s[ri, r_:r_ + 8, :] = tt[8 * g:8 * g + 8]

    zpad = jnp.zeros((16, 128), f32)

    def pad_bf(v):
        return jnp.concatenate([v, zpad], axis=0).astype(bf)

    def mat(k1, j):
        return mf[k1, 128 * j:128 * j + 128, :]

    def s_forward(t, k1):
        a, b = z_s[t, 0, k1], z_s[t, 1, k1]
        m1 = d_nt(mat(k1, 0), pad_bf(a + b))
        m2 = d_nt(mat(k1, 1), pad_bf(a))
        m3 = d_nt(mat(k1, 2), pad_bf(b))
        y_s[0, t, k1] = m1 - m3
        y_s[1, t, k1] = m1 + m2

    def s_inverse(t, k1):
        def half(v):
            if t == 0:
                return pltpu.bitcast(v << np.uint32(16), f32)
            return pltpu.bitcast(v & np.uint32(0xFFFF0000), f32)
        wr = half(wt_s[0, pl.ds(k1, 128, stride=17), :])
        wi = half(wt_s[1, pl.ds(k1, 128, stride=17), :])
        yr0, yi0 = y_s[0, t, k1], y_s[1, t, k1]
        yr, yi = yr0 * wr - yi0 * wi, yr0 * wi + yi0 * wr
        m1 = d_tn(mat(k1, 0), (yr + yi).astype(bf))
        m2 = d_tn(mat(k1, 1), yi.astype(bf))
        m3 = d_tn(mat(k1, 2), yr.astype(bf))
        u_s[0, t, 128 * k1:128 * k1 + 128, :] = m1 + m2
        u_s[1, t, 128 * k1:128 * k1 + 128, :] = m1 - m3

    lane_even = (lax.broadcasted_iota(jnp.int32, (128, 128), 1) & 1) == 0

    def d_inverse_even(ai):
        rs = slice(128 * ai, 128 * ai + 128)
        re, im = u_s[0, 0, rs, :], u_s[1, 0, rs, :]
        t0 = jnp.where(lane_even, re, pltpu.roll(im, 1, 1)).astype(bf)
        t2 = jnp.where(lane_even, pltpu.roll(re, 127, 1), im).astype(bf)
        v0, v2 = d_nt(lie[0], t0), d_nt(lie[1], t2)
        ve[:, rs] = jnp.concatenate([v0 + v2, v0 - v2], axis=0)

    def d_inverse_odd(ai):
        rs = slice(128 * ai, 128 * ai + 128)
        v = jnp.concatenate([u_s[0, 1, rs, :], u_s[1, 1, rs, :]], axis=1).astype(bf)
        return d_nt(lio[...], v)

    def build_b(j, r0):
        cs = slice(256 * j, 256 * j + 256)
        lo, hi = slice(r0, r0 + 32), slice(H + r0, H + r0 + 32)
        gl, gh = wg[lo, cs].astype(f32), wg[hi, cs].astype(f32)
        ul, uh = wu[lo, cs].astype(f32), wu[hi, cs].astype(f32)
        for i, v in enumerate((gl + uh, ul - uh, gh - gl, gl + ul, gh + uh)):
            bw[i, lo, cs] = v.astype(bf)

    def build_a(j0, r0):
        js = [j for j in (j0, j0 + 1) if j < 7]
        cs = slice(128 * j0, 128 * j0 + 128 * len(js))
        lo = [wd[r0:r0 + 32, 256 * j:256 * j + 256].astype(f32) for j in js]
        hi = [wd[H + r0:H + r0 + 32, 256 * j:256 * j + 256].astype(f32) for j in js]

        def cat(vs, odd):
            return jnp.concatenate([v[:, 128 * odd:128 * odd + 128] for v in vs], axis=1)
        a11, a12, a21, a22 = cat(lo, 0), cat(lo, 1), cat(hi, 0), cat(hi, 1)
        for i, v in enumerate((a11 + a22, a21 + a22, a11 + a12, a21 - a11, a12 - a22)):
            aw[i, r0:r0 + 32, cs] = v.astype(bf)

    def prep_norm(c, q):
        ai = 4 * c + q
        cs, qs = slice(128 * ai, 128 * ai + 128), slice(128 * q, 128 * q + 128)
        vo = d_inverse_odd(ai)
        s1 = s2 = None
        for r0 in range(0, H, 32):
            v0, v1 = ve[r0:r0 + 32, cs], vo[r0:r0 + 32]
            hl = (xs[r0:r0 + 32, cs].astype(f32) + (v0 + v1)).astype(bf)
            hh = (xs[H + r0:H + r0 + 32, cs].astype(f32) + (v0 - v1)).astype(bf)
            hb[c % 3, r0:r0 + 32, qs] = hl
            hb[c % 3, H + r0:H + r0 + 32, qs] = hh
            a, b = hl.astype(f32), hh.astype(f32)
            t1, t2 = a + b, a * a + b * b
            s1 = t1 if s1 is None else s1 + t1
            s2 = t2 if s2 is None else s2 + t2
        m = jnp.sum(s1, axis=0, keepdims=True) * (1.0 / D)
        var = jnp.sum(s2, axis=0, keepdims=True) * (1.0 / D) - m * m
        rr = lax.rsqrt(jnp.maximum(var, 0.0) + EPS)
        for r0 in range(0, D, 32):
            lnf[r0:r0 + 32, qs] = (hb[c % 3, r0:r0 + 32, qs].astype(f32) - m) * rr

    def prep_sums(c, q):
        qa, qb = slice(128 * q, 128 * q + 128), slice(TH + 128 * q, TH + 128 * q + 128)
        l11, l12, l21, l22 = lnf[0:H, qa], lnf[H:D, qa], lnf[0:H, qb], lnf[H:D, qb]
        for i, a in enumerate((l11 + l22, l21 + l22, l11, l22, l11 + l12, l21 - l11, l12 - l22)):
            al[c % 2, i, qa, :] = a.T.astype(bf)

    def prep_tasks(c):
        out = []
        for q in range(2):
            out += [P(prep_norm, c, q), P(prep_norm, c, 2 + q), P(prep_sums, c, q)]
        return out

    def gate_up(c, j):
        cs, lo = slice(256 * j, 256 * j + 256), slice(128 * j, 128 * j + 128)

        def rhs(i):
            if i == 1:
                return wg[0:H, cs]
            if i == 4:
                return wu[H:D, cs]
            return bw[{0: 0, 2: 1, 3: 2, 5: 3, 6: 4}[i], :, cs]
        m = [None] * 7
        for i in (1, 4, 2, 0, 3, 6, 5):
            m[i] = d_nn(al[c % 2, i], rhs(i))
            yield
        ha = (m[0] + m[3] - m[4] + m[6]) * (m[2] + m[4])
        hh = (m[1] + m[3]) * (m[0] - m[1] + m[2] + m[5])
        alo, ahi, blo, bhi = ha[:, 0:128], ha[:, 128:256], hh[:, 0:128], hh[:, 128:256]
        cb = (alo + bhi, alo, blo - bhi, ahi - alo, bhi, alo + blo, ahi + bhi)
        for p in range(3):
            bc[p, :, cs] = jnp.concatenate([cb[2 * p], cb[2 * p + 1]], axis=1).astype(bf)
        bc[3, :, lo] = cb[6].astype(bf)

    outs = []

    def down(c):
        def lhs(i):
            if i == 2:
                return jnp.concatenate([wd[0:H, 256 * j:256 * j + 128] for j in range(7)], axis=1)
            if i == 3:
                return jnp.concatenate([wd[H:D, 256 * j + 128:256 * j + 256] for j in range(7)], axis=1)
            return aw[{0: 0, 1: 1, 4: 2, 5: 3, 6: 4}[i]]

        def rhs(i):
            if i == 6:
                return bc[3, :, 0:FH]
            off = 128 * (i % 2)
            return jnp.concatenate(
                [bc[i // 2, :, 256 * j + off:256 * j + off + 128] for j in range(7)], axis=1)

        def prod(i):
            return d_nt(lhs(i), rhs(i))

        def res(r0, c0):
            return hb[c % 3, r0:r0 + H, c0:c0 + TH].astype(f32)

        def emit(r0, c0, v):
            cols = slice(c * T + c0, c * T + c0 + TH)
            ob[r0:r0 + H, cols] = v.astype(bf)
            d = dma(ob.at[r0:r0 + H, cols], o_h.at[r0:r0 + H, cols])
            d.start()
            outs.append(d)

        m5 = prod(4)
        yield
        c11, c12 = res(0, 0) - m5, res(0, TH) + m5
        m3 = prod(2)
        yield
        emit(0, TH, c12 + m3)
        c22 = res(H, TH) + m3
        m2 = prod(1)
        yield
        c21, c22 = res(H, 0) + m2, c22 - m2
        m4 = prod(3)
        yield
        emit(H, 0, c21 + m4)
        c11 = c11 + m4
        m1 = prod(0)
        yield
        c11, c22 = c11 + m1, c22 + m1
        m7 = prod(6)
        yield
        emit(0, 0, c11 + m7)
        m6 = prod(5)
        yield
        emit(H, TH, c22 + m6)

    radix16_fwd(0, range(14))

    for d in d_nq + d_w[0]:
        d.wait()
    _interleave([_step(s_forward, 0, k1) for k1 in range(16)],
                [P(filter_t, 0)] + [P(radix16_fwd, 1, [g]) for g in range(14)])

    for d in d_w[1] + d_w[2]:
        d.wait()
    _interleave([_step(s_forward, 1, k1) for k1 in range(8)], [P(filter_t, 1), P(filter_t, 2)])
    for d in d_w[3]:
        d.wait()
    _interleave([_step(s_forward, 1, k1) for k1 in range(8, 16)], [P(filter_t, 3)])

    for k1 in range(16):
        s_inverse(0, k1)
    _interleave([_step(s_inverse, 1, k1) for k1 in range(16)],
                [P(radix16_inv, 0, g) for g in range(16)])

    for d in d_li:
        d.wait()
    _interleave([_step(d_inverse_even, ai) for ai in range(16)],
                [P(radix16_inv, 1, g) for g in range(16)])

    for d in d_gu:
        d.wait()
    for j in range(7):
        for r0 in range(0, H, 32):
            build_b(j, r0)
    for task in prep_tasks(0):
        task()

    for c in range(4):
        if c == 0:
            d_wd.wait()
            for j0 in range(0, 7, 2):
                for r0 in range(0, H, 32):
                    build_a(j0, r0)
        _interleave([(P(gate_up, c, j), 7) for j in range(7)], prep_tasks(c + 1) if c < 3 else [])
        _interleave([(P(down, c), 7)], [])

    for d in outs:
        d.wait()


@jax.jit
def pallas_sequential_preLN__spectral_gfnet__glu_gated_bilinear__prompt_kernel(
    A_x: jax.Array,
    A_w_r: jax.Array,
    A_w_i: jax.Array,
    B_x: jax.Array,
    B_w_gate: jax.Array,
    B_w_up: jax.Array,
    B_w_down: jax.Array,
):
    del B_x
    li_odd, li_even = _inverse_d_matrices()
    hbm = pl.BlockSpec(memory_space=pltpu.HBM)
    vmem = pltpu.VMEM
    out = pl.pallas_call(
        _kernel,
        out_shape=jax.ShapeDtypeStruct((D, S), bf),
        in_specs=[hbm] * 8,
        out_specs=hbm,
        scratch_shapes=[
            vmem((D, S), bf),
            vmem((2, H, S), bf),
            vmem((2, 1, S), bf),
            vmem((D, F), bf),
            vmem((D, F), bf),
            vmem((D, F), bf),
            vmem((2, H, H), bf),
            vmem((H, 256), bf),
            vmem((2, 112, 128), bf),
            vmem((16, 384, 128), bf),
            vmem((2, 2, 16, 112, 128), f32),
            vmem((2, 2, 16, 128, 128), f32),
            vmem((2, 17 * 128 + 16, 128), u32),
            vmem((2, 2, S, 128), f32),
            vmem((H, S), f32),
            vmem((D, T), f32),
            vmem((2, 7, TH, H), bf),
            vmem((3, D, T), bf),
            vmem((D, S), bf),
            vmem((5, H, F), bf),
            vmem((5, H, FH), bf),
            vmem((4, TH, F), bf),
            pltpu.SemaphoreType.DMA((48,)),
        ],
        compiler_params=pltpu.CompilerParams(vmem_limit_bytes=100 * 1024 * 1024),
    )(A_x.reshape(S, D).T, A_w_r.T, A_w_i.T, B_w_gate, B_w_up, B_w_down.T, li_odd, li_even)
    return out.T.reshape(1, S, D)
```

```python
import functools
import math

import jax
import jax.numpy as jnp
import ml_dtypes
import numpy as np
from jax import lax
import jax.experimental.pallas as pl
import jax.experimental.pallas.tpu as pltpu

S, D, F = 2048, 448, 1792
H = D // 2
FH = F // 2
T = 512
TH = T // 2
EPS = 1e-5

bf = jnp.bfloat16
f32 = jnp.float32
u32 = jnp.uint32
P = functools.partial

_NT = (((1,), (1,)), ((), ()))
_TN = (((0,), (0,)), ((), ()))


def d_nn(a, b):
    return jnp.dot(a, b, preferred_element_type=f32)


def d_nt(a, b):
    return lax.dot_general(a, b, _NT, preferred_element_type=f32)


def d_tn(a, b):
    return lax.dot_general(a, b, _TN, preferred_element_type=f32)


def _cos_sin(num, den):
    a = 2 * np.pi * np.mod(num, den) / den
    c, s = np.cos(a), np.sin(a)
    return np.where(np.abs(c) < 1e-12, 0, c), np.where(np.abs(s) < 1e-12, 0, s)


def _inverse_d_matrices():
    k_even = 2 * np.arange(112)
    k_even[0] = H
    k_odd = 2 * np.arange(112) + 1
    scale = 1.0 / (D * S)
    odd = np.zeros((H, 256))
    c, s = _cos_sin(np.arange(H)[:, None] * k_odd[None, :], D)
    odd[:, :112] = 2 * scale * c
    odd[:, 128:240] = -2 * scale * s
    even = np.zeros((2, 112, 128))
    for j, k in enumerate((k_even[0::2], k_even[1::2])):
        w = np.where(k == H, 1.0, 2.0) * scale
        c, s = _cos_sin(np.arange(112)[:, None] * k[None, :], D)
        even[j, :, 0:112:2] = c * w
        even[j, :, 1:112:2] = -s * w
    return odd.astype(ml_dtypes.bfloat16), even.astype(ml_dtypes.bfloat16)


def _cadd(a, b):
    return a[0] + b[0], a[1] + b[1]


def _csub(a, b):
    return a[0] - b[0], a[1] - b[1]


def _fft4(x, inv):
    t0, t1 = _cadd(x[0], x[2]), _csub(x[0], x[2])
    t2, t3 = _cadd(x[1], x[3]), _csub(x[1], x[3])
    mi = (t1[0] + t3[1], t1[1] - t3[0])
    pi = (t1[0] - t3[1], t1[1] + t3[0])
    return [_cadd(t0, t2), pi if inv else mi, _csub(t0, t2), mi if inv else pi]


def _tw16(x, e, inv):
    a, b = x
    if e == 0:
        return x
    if e == 4:
        return (-b, a) if inv else (b, -a)
    c = math.cos(2 * math.pi * e / 16)
    s = math.sin(2 * math.pi * e / 16) * (1 if inv else -1)
    if e in (2, 6):
        r = abs(c)
        if c > 0 and s > 0:
            return (a - b) * r, (a + b) * r
        if c > 0 and s < 0:
            return (a + b) * r, (b - a) * r
        if c < 0 and s > 0:
            return (a + b) * (-r), (a - b) * r
        return (b - a) * r, (a + b) * (-r)
    return a * c - b * s, b * c + a * s


def _fft16(x, inv):
    t = [None] * 16
    for a0 in range(4):
        y = _fft4([x[4 * a1 + a0] for a1 in range(4)], inv)
        for k0 in range(4):
            t[4 * a0 + k0] = _tw16(y[k0], a0 * k0, inv)
    out = [None] * 16
    for k0 in range(4):
        y = _fft4([t[4 * a0 + k0] for a0 in range(4)], inv)
        for k in range(4):
            out[k0 + 4 * k] = y[k]
    return out


def _interleave(main, side):
    n = sum(cnt for _, cnt in main)
    i = done = 0
    for fn, cnt in main:
        g = fn()
        for _ in range(cnt):
            next(g)
            i += 1
            while done < len(side) and done < len(side) * i / n:
                side[done]()
                done += 1
        for _ in g:
            pass
    while done < len(side):
        side[done]()
        done += 1


def _step(fn, *args):
    def gen():
        fn(*args)
        yield
    return gen, 1


def _kernel(x_h, wr_h, wi_h, wg_h, wu_h, wd_h, lo_h, le_h, o_h,
            xs, wraw, nyq, wg, wu, wd, ldf, lio, lie, mf, z_s, y_s, wt_s, u_s, ve, lnf,
            al, hb, ob, bw, aw, bc, sem):
    sem_ids = iter(range(48))

    def dma(src, dst):
        return pltpu.make_async_copy(src, dst, sem.at[next(sem_ids)])

    d_x = [dma(x_h.at[:, 512 * c:512 * c + 512], xs.at[:, 512 * c:512 * c + 512]) for c in range(4)]
    d_nq = [dma(wr_h.at[H:H + 1, :], nyq.at[0]), dma(wi_h.at[H:H + 1, :], nyq.at[1])]
    d_w = [[dma(w.at[0:H, 512 * c:512 * c + 512], wraw.at[i, :, 512 * c:512 * c + 512])
            for i, w in enumerate((wr_h, wi_h))] for c in range(4)]
    d_li = [dma(lo_h, lio), dma(le_h, lie)]
    d_gu = [dma(wg_h, wg), dma(wu_h, wu)]
    d_wd = dma(wd_h, wd)
    for d in d_x + d_nq + [d for ds in d_w for d in ds] + d_li + d_gu + [d_wd]:
        d.start()

    r = lax.broadcasted_iota(jnp.int32, (128, 128), 0)
    c_ = lax.broadcasted_iota(jnp.int32, (128, 128), 1)
    ang = ((r * c_) & 127).astype(f32) * (2 * math.pi / 128)
    c0, s0 = jnp.cos(ang), -jnp.sin(ang)
    r2 = lax.broadcasted_iota(jnp.int32, (16, 128), 0)
    c2 = lax.broadcasted_iota(jnp.int32, (16, 128), 1)
    a2 = (r2 * c2).astype(f32) * (2 * math.pi / S)
    tc, ts = jnp.cos(a2), -jnp.sin(a2)
    for k1 in range(16):
        if k1 == 0:
            cm, sm = c0, s0
        else:
            a, b = tc[k1:k1 + 1, :], ts[k1:k1 + 1, :]
            cm, sm = c0 * a - s0 * b, c0 * b + s0 * a
        for j, m in enumerate((cm, sm - cm, cm + sm)):
            mf[k1, 128 * j:128 * j + 128, :] = m.astype(bf)

    def cs_d(n):
        n = n.astype(f32)
        n = n - jnp.floor(n * (1.0 / D)) * D
        a_ = n * (2 * math.pi / D)
        return jnp.cos(a_), -jnp.sin(a_)

    stc, sts = cs_d(16 * lax.broadcasted_iota(jnp.int32, (16, H), 0)
                    * lax.broadcasted_iota(jnp.int32, (16, H), 1))
    s8 = lax.broadcasted_iota(jnp.int32, (8, H), 0)
    d8 = lax.broadcasted_iota(jnp.int32, (8, H), 1)
    for t in range(2):
        bc_, bs_ = cs_d((2 * s8 + t) * d8)
        cr, sr = [], []
        for g in range(14):
            if g == 0:
                c1, s1 = bc_, bs_
            else:
                sc, ss = stc[g:g + 1, :], sts[g:g + 1, :]
                c1, s1 = bc_ * sc - bs_ * ss, bc_ * ss + bs_ * sc
            if g == 0 and t == 0:
                c1 = jnp.where(s8 == 0, (1 - 2 * (d8 & 1)).astype(f32), c1)
                s1 = jnp.where(s8 == 0, 0.0, s1)
            cr.append(c1)
            sr.append(s1)
        ldf[t, 0:112, :] = jnp.concatenate(cr, axis=0).astype(bf)
        ldf[t, 112:H, :] = jnp.concatenate(sr, axis=0).astype(bf)

    def d_forward(ai):
        cs = slice(128 * ai, 128 * ai + 128)
        lo, hi = xs[0:H, cs].astype(f32), xs[H:D, cs].astype(f32)
        o = lo - hi
        obf = o.astype(bf)
        e = lo + hi
        so = jnp.sum(o * o, axis=0, keepdims=True)
        ec = e - jnp.sum(e, axis=0, keepdims=True) * (1.0 / H)
        ebf = ec.astype(bf)
        ss = so + jnp.sum(ec * ec, axis=0, keepdims=True)
        rr = lax.rsqrt(ss * (0.5 / D) + EPS)
        for t, v in enumerate((ebf, obf)):
            z = d_nn(ldf[t], v) * rr
            z_s[t, 0, ai] = z[:112]
            z_s[t, 1, ai] = z[112:]

    for c in range(4):
        d_x[c].wait()
        for ai in range(4 * c, 4 * c + 4):
            d_forward(ai)

    def radix16_fwd(t, groups):
        for g in groups:
            rows = slice(8 * g, 8 * g + 8)
            y = _fft16([(z_s[t, 0, a, rows, :], z_s[t, 1, a, rows, :]) for a in range(16)], False)
            for k in range(16):
                z_s[t, 0, k, rows, :] = y[k][0]
                z_s[t, 1, k, rows, :] = y[k][1]

    def radix16_inv(t, g):
        def rows(a):
            return slice(128 * a + 8 * g, 128 * a + 8 * g + 8)
        y = _fft16([(u_s[0, t, rows(k), :], u_s[1, t, rows(k), :]) for k in range(16)], True)
        for a in range(16):
            u_s[0, t, rows(a), :] = y[a][0]
            u_s[1, t, rows(a), :] = y[a][1]

    def filter_t(c):
        for ri in range(2):
            for p in range(4 * c, 4 * c + 4):
                cs = slice(128 * p, 128 * p + 128)
                w = pltpu.bitcast(wraw[ri, :, cs], u32)
                nq = lax.shift_right_logical(
                    pltpu.bitcast(nyq[ri, :, cs].astype(f32), u32), np.uint32(16))
                row0 = lax.broadcasted_iota(jnp.int32, (8, 128), 0) == 0
                first = jnp.where(row0, (w[0:8] & np.uint32(0xFFFF0000)) | nq, w[0:8])
                tt = jnp.concatenate([first, w[8:112], jnp.zeros((16, 128), u32)], axis=0).T
                for g in range(16):
                    r_ = 17 * (8 * p + g // 2) + 8 * (g % 2)
                    wt_s[ri, r_:r_ + 8, :] = tt[8 * g:8 * g + 8]

    zpad = jnp.zeros((16, 128), f32)

    def pad_bf(v):
        return jnp.concatenate([v, zpad], axis=0).astype(bf)

    def mat(k1, j):
        return mf[k1, 128 * j:128 * j + 128, :]

    def s_forward(t, k1):
        a, b = z_s[t, 0, k1], z_s[t, 1, k1]
        m1 = d_nt(mat(k1, 0), pad_bf(a + b))
        m2 = d_nt(mat(k1, 1), pad_bf(a))
        m3 = d_nt(mat(k1, 2), pad_bf(b))
        y_s[0, t, k1] = m1 - m3
        y_s[1, t, k1] = m1 + m2

    def s_inverse(t, k1):
        def half(v):
            if t == 0:
                return pltpu.bitcast(v << np.uint32(16), f32)
            return pltpu.bitcast(v & np.uint32(0xFFFF0000), f32)
        wr = half(wt_s[0, pl.ds(k1, 128, stride=17), :])
        wi = half(wt_s[1, pl.ds(k1, 128, stride=17), :])
        yr0, yi0 = y_s[0, t, k1], y_s[1, t, k1]
        yr, yi = yr0 * wr - yi0 * wi, yr0 * wi + yi0 * wr
        m1 = d_tn(mat(k1, 0), (yr + yi).astype(bf))
        m2 = d_tn(mat(k1, 1), yi.astype(bf))
        m3 = d_tn(mat(k1, 2), yr.astype(bf))
        u_s[0, t, 128 * k1:128 * k1 + 128, :] = m1 + m2
        u_s[1, t, 128 * k1:128 * k1 + 128, :] = m1 - m3

    lane_even = (lax.broadcasted_iota(jnp.int32, (128, 128), 1) & 1) == 0

    def d_inverse_even(ai):
        rs = slice(128 * ai, 128 * ai + 128)
        re, im = u_s[0, 0, rs, :], u_s[1, 0, rs, :]
        t0 = jnp.where(lane_even, re, pltpu.roll(im, 1, 1)).astype(bf)
        t2 = jnp.where(lane_even, pltpu.roll(re, 127, 1), im).astype(bf)
        v0, v2 = d_nt(lie[0], t0), d_nt(lie[1], t2)
        ve[:, rs] = jnp.concatenate([v0 + v2, v0 - v2], axis=0)

    def d_inverse_odd(ai):
        rs = slice(128 * ai, 128 * ai + 128)
        v = jnp.concatenate([u_s[0, 1, rs, :], u_s[1, 1, rs, :]], axis=1).astype(bf)
        return d_nt(lio[...], v)

    def tiles(g, u, odd):
        return jnp.concatenate([g[:, 128 * odd:128 * odd + 128], u[:, 128 * odd:128 * odd + 128]], axis=1)

    def build_b(j, r0):
        cs = slice(256 * j, 256 * j + 256)
        lo, hi = slice(r0, r0 + 32), slice(H + r0, H + r0 + 32)
        gl, gh = wg[lo, cs].astype(f32), wg[hi, cs].astype(f32)
        ul, uh = wu[lo, cs].astype(f32), wu[hi, cs].astype(f32)
        b11, b12, b21, b22 = tiles(gl, ul, 0), tiles(gl, ul, 1), tiles(gh, uh, 0), tiles(gh, uh, 1)
        for i, v in enumerate((b11 + b22, b12 - b22, b21 - b11, b11 + b12, b21 + b22)):
            bw[i, lo, cs] = v.astype(bf)

    def build_a(j0, r0):
        js = [j for j in (j0, j0 + 1) if j < 7]
        cs = slice(128 * j0, 128 * j0 + 128 * len(js))
        lo = [wd[r0:r0 + 32, 256 * j:256 * j + 256].astype(f32) for j in js]
        hi = [wd[H + r0:H + r0 + 32, 256 * j:256 * j + 256].astype(f32) for j in js]

        def cat(vs, odd):
            return jnp.concatenate([v[:, 128 * odd:128 * odd + 128] for v in vs], axis=1)
        a11, a12, a21, a22 = cat(lo, 0), cat(lo, 1), cat(hi, 0), cat(hi, 1)
        for i, v in enumerate((a11 + a22, a21 + a22, a11 + a12, a21 - a11, a12 - a22)):
            aw[i, r0:r0 + 32, cs] = v.astype(bf)

    def prep_norm(c, q):
        ai = 4 * c + q
        cs, qs = slice(128 * ai, 128 * ai + 128), slice(128 * q, 128 * q + 128)
        vo = d_inverse_odd(ai)
        s1 = s2 = None
        for r0 in range(0, H, 32):
            v0, v1 = ve[r0:r0 + 32, cs], vo[r0:r0 + 32]
            hl = (xs[r0:r0 + 32, cs].astype(f32) + (v0 + v1)).astype(bf)
            hh = (xs[H + r0:H + r0 + 32, cs].astype(f32) + (v0 - v1)).astype(bf)
            hb[c % 3, r0:r0 + 32, qs] = hl
            hb[c % 3, H + r0:H + r0 + 32, qs] = hh
            a, b = hl.astype(f32), hh.astype(f32)
            t1, t2 = a + b, a * a + b * b
            s1 = t1 if s1 is None else s1 + t1
            s2 = t2 if s2 is None else s2 + t2
        m = jnp.sum(s1, axis=0, keepdims=True) * (1.0 / D)
        var = jnp.sum(s2, axis=0, keepdims=True) * (1.0 / D) - m * m
        rr = lax.rsqrt(jnp.maximum(var, 0.0) + EPS)
        for r0 in range(0, D, 32):
            lnf[r0:r0 + 32, qs] = (hb[c % 3, r0:r0 + 32, qs].astype(f32) - m) * rr

    def prep_sums(c, q):
        qa, qb = slice(128 * q, 128 * q + 128), slice(TH + 128 * q, TH + 128 * q + 128)
        l11, l12, l21, l22 = lnf[0:H, qa], lnf[H:D, qa], lnf[0:H, qb], lnf[H:D, qb]
        for i, a in enumerate((l11 + l22, l21 + l22, l11, l22, l11 + l12, l21 - l11, l12 - l22)):
            al[c % 2, i, qa, :] = a.T.astype(bf)

    def prep_tasks(c):
        out = []
        for q in range(2):
            out += [P(prep_norm, c, q), P(prep_norm, c, 2 + q), P(prep_sums, c, q)]
        return out

    def gate_up(c, j):
        cs, lo = slice(256 * j, 256 * j + 256), slice(128 * j, 128 * j + 128)
        ev, od = slice(256 * j, 256 * j + 128), slice(256 * j + 128, 256 * j + 256)

        def rhs(i):
            if i == 1:
                return jnp.concatenate([wg[0:H, ev], wu[0:H, ev]], axis=1)
            if i == 4:
                return jnp.concatenate([wg[H:D, od], wu[H:D, od]], axis=1)
            return bw[{0: 0, 2: 1, 3: 2, 5: 3, 6: 4}[i], :, cs]

        def glu(v):
            return v[:, 0:128] * v[:, 128:256]
        m = [None] * 7
        for i in (1, 4, 2, 0, 3, 6, 5):
            m[i] = d_nn(al[c % 2, i], rhs(i))
            yield
        alo, ahi = glu(m[0] + m[3] - m[4] + m[6]), glu(m[2] + m[4])
        blo, bhi = glu(m[1] + m[3]), glu(m[0] - m[1] + m[2] + m[5])
        cb = (alo + bhi, alo, blo - bhi, ahi - alo, bhi, alo + blo, ahi + bhi)
        for p in range(3):
            bc[p, :, cs] = jnp.concatenate([cb[2 * p], cb[2 * p + 1]], axis=1).astype(bf)
        bc[3, :, lo] = cb[6].astype(bf)

    outs = []

    def down(c):
        def lhs(i):
            if i == 2:
                return jnp.concatenate([wd[0:H, 256 * j:256 * j + 128] for j in range(7)], axis=1)
            if i == 3:
                return jnp.concatenate([wd[H:D, 256 * j + 128:256 * j + 256] for j in range(7)], axis=1)
            return aw[{0: 0, 1: 1, 4: 2, 5: 3, 6: 4}[i]]

        def rhs(i):
            if i == 6:
                return bc[3, :, 0:FH]
            off = 128 * (i % 2)
            return jnp.concatenate(
                [bc[i // 2, :, 256 * j + off:256 * j + off + 128] for j in range(7)], axis=1)

        def prod(i):
            return d_nt(lhs(i), rhs(i))

        def res(r0, c0):
            return hb[c % 3, r0:r0 + H, c0:c0 + TH].astype(f32)

        def emit(r0, c0, v):
            cols = slice(c * T + c0, c * T + c0 + TH)
            ob[r0:r0 + H, cols] = v.astype(bf)
            d = dma(ob.at[r0:r0 + H, cols], o_h.at[r0:r0 + H, cols])
            d.start()
            outs.append(d)

        m5 = prod(4)
        yield
        c11, c12 = res(0, 0) - m5, res(0, TH) + m5
        m3 = prod(2)
        yield
        emit(0, TH, c12 + m3)
        c22 = res(H, TH) + m3
        m2 = prod(1)
        yield
        c21, c22 = res(H, 0) + m2, c22 - m2
        m4 = prod(3)
        yield
        emit(H, 0, c21 + m4)
        c11 = c11 + m4
        m1 = prod(0)
        yield
        c11, c22 = c11 + m1, c22 + m1
        m7 = prod(6)
        yield
        emit(0, 0, c11 + m7)
        m6 = prod(5)
        yield
        emit(H, TH, c22 + m6)

    radix16_fwd(0, range(14))

    for d in d_nq + d_w[0]:
        d.wait()
    _interleave([_step(s_forward, 0, k1) for k1 in range(16)],
                [P(filter_t, 0)] + [P(radix16_fwd, 1, [g]) for g in range(14)])

    for d in d_w[1] + d_w[2]:
        d.wait()
    _interleave([_step(s_forward, 1, k1) for k1 in range(8)], [P(filter_t, 1), P(filter_t, 2)])
    for d in d_w[3]:
        d.wait()
    _interleave([_step(s_forward, 1, k1) for k1 in range(8, 16)], [P(filter_t, 3)])

    for k1 in range(16):
        s_inverse(0, k1)
    _interleave([_step(s_inverse, 1, k1) for k1 in range(16)],
                [P(radix16_inv, 0, g) for g in range(16)])

    for d in d_li:
        d.wait()
    _interleave([_step(d_inverse_even, ai) for ai in range(16)],
                [P(radix16_inv, 1, g) for g in range(16)])

    for d in d_gu:
        d.wait()
    for j in range(7):
        for r0 in range(0, H, 32):
            build_b(j, r0)
    for task in prep_tasks(0):
        task()

    for c in range(4):
        if c == 0:
            d_wd.wait()
            for j0 in range(0, 7, 2):
                for r0 in range(0, H, 32):
                    build_a(j0, r0)
        _interleave([(P(gate_up, c, j), 7) for j in range(7)], prep_tasks(c + 1) if c < 3 else [])
        _interleave([(P(down, c), 7)], [])

    for d in outs:
        d.wait()


@jax.jit
def pallas_sequential_preLN__spectral_gfnet__glu_gated_bilinear__prompt_kernel(
    A_x: jax.Array,
    A_w_r: jax.Array,
    A_w_i: jax.Array,
    B_x: jax.Array,
    B_w_gate: jax.Array,
    B_w_up: jax.Array,
    B_w_down: jax.Array,
):
    del B_x
    li_odd, li_even = _inverse_d_matrices()
    hbm = pl.BlockSpec(memory_space=pltpu.HBM)
    vmem = pltpu.VMEM
    out = pl.pallas_call(
        _kernel,
        out_shape=jax.ShapeDtypeStruct((D, S), bf),
        in_specs=[hbm] * 8,
        out_specs=hbm,
        scratch_shapes=[
            vmem((D, S), bf),
            vmem((2, H, S), bf),
            vmem((2, 1, S), bf),
            vmem((D, F), bf),
            vmem((D, F), bf),
            vmem((D, F), bf),
            vmem((2, H, H), bf),
            vmem((H, 256), bf),
            vmem((2, 112, 128), bf),
            vmem((16, 384, 128), bf),
            vmem((2, 2, 16, 112, 128), f32),
            vmem((2, 2, 16, 128, 128), f32),
            vmem((2, 17 * 128 + 16, 128), u32),
            vmem((2, 2, S, 128), f32),
            vmem((H, S), f32),
            vmem((D, T), f32),
            vmem((2, 7, TH, H), bf),
            vmem((3, D, T), bf),
            vmem((D, S), bf),
            vmem((5, H, F), bf),
            vmem((5, H, FH), bf),
            vmem((4, TH, F), bf),
            pltpu.SemaphoreType.DMA((48,)),
        ],
        compiler_params=pltpu.CompilerParams(vmem_limit_bytes=100 * 1024 * 1024),
    )(A_x.reshape(S, D).T, A_w_r.T, A_w_i.T, B_w_gate, B_w_up, B_w_down.T, li_odd, li_even)
    return out.T.reshape(1, S, D)
```
